```python
import jax
import jax.numpy as jnp

def _softmax(x, axis=-1):
    return jax.nn.softmax(x, axis=axis)
def _gelu(x):
    return jax.nn.gelu(x, approximate=True)
def _silu(x):
    return jax.nn.silu(x)
def _sigmoid(x):
    return jax.nn.sigmoid(x)
def _layernorm(x, axis=-1, eps=1e-5):
    m = jnp.mean(x, axis=axis, keepdims=True)
    v = jnp.var(x, axis=axis, keepdims=True)
    return (x - m) / jnp.sqrt(v + eps)
def _scatter_add(tgt, idx, src, axis=0):
    return tgt.at[idx].add(src)
def _segment_sum(src, seg, n):
    return jax.ops.segment_sum(src, seg, n)
class _Rng:
    def __init__(self, key):
        self._k = key
    def _next(self):
        self._k, sub = jax.random.split(self._k)
        return sub
    def normal(self, shape):
        return jax.random.normal(self._next(), shape, dtype=jnp.bfloat16)
    def randint(self, lo, hi, shape):
        return jax.random.randint(self._next(), shape, lo, hi, dtype=jnp.int32)
    def uniform(self, shape, lo=0.0, hi=1.0):
        return jax.random.uniform(self._next(), shape, jnp.bfloat16, lo, hi)
    def permutation(self, n):
        return jax.random.permutation(self._next(), n)


kernel_name = 'recurrent_scan__compressed_kv_cla__moe_arch_mod__decode'

def setup_inputs():
    _rng = _Rng(jax.random.key(int.from_bytes(__import__("os").urandom(4), "little")))
    _w = (lambda a: (lambda t: t.astype(jnp.bfloat16) if jnp.issubdtype(t.dtype, jnp.floating) else t)(jnp.asarray(a)))
    def _A_setup():
        B, H, Sq, Sk, D, M = 4, 32, 1, 4096, 128, 576
        Dc = 4 * D
        return {
            "x": _w((lambda *s: _rng.normal(s) * 0.05)(B, Sq, M)),
            "c_kv": _w((lambda *s: _rng.normal(s) * 0.05)(B, Sk, Dc)),
            "w_q": _w((lambda *s: _rng.normal(s) * 0.05)(M, H, D) * (M ** -0.5)),
            "w_uk": _w((lambda *s: _rng.normal(s) * 0.05)(Dc, H, D) * (Dc ** -0.5)),
            "w_uv": _w((lambda *s: _rng.normal(s) * 0.05)(Dc, H, D) * (Dc ** -0.5)),
            "w_o": _w((lambda *s: _rng.normal(s) * 0.05)(H, D, M) * ((H * D) ** -0.5)),
        }
    _A_in = _A_setup()

    def _B_setup():
        B, S, D, F, C = 4, 1, 576, 4608, 1
        return {
            "x": _w((lambda *s: _rng.normal(s) * 0.05)(B, S, D)),
            "w_r": _w((lambda *s: _rng.normal(s) * 0.05)(D)),
            "w_gate": _w((lambda *s: _rng.normal(s) * 0.05)(D, F)),
            "w_up": _w((lambda *s: _rng.normal(s) * 0.05)(D, F)),
            "w_down": _w((lambda *s: _rng.normal(s) * 0.05)(F, D)),
        }
    _B_in = _B_setup()

    return {
        "A_x": _A_in["x"],
        "A_c_kv": _A_in["c_kv"],
        "A_w_q": _A_in["w_q"],
        "A_w_uk": _A_in["w_uk"],
        "A_w_uv": _A_in["w_uv"],
        "A_w_o": _A_in["w_o"],
        "B_x": _B_in["x"],
        "B_w_r": _B_in["w_r"],
        "B_w_gate": _B_in["w_gate"],
        "B_w_up": _B_in["w_up"],
        "B_w_down": _B_in["w_down"],
    }

def reference(A_x, A_c_kv, A_w_q, A_w_uk, A_w_uv, A_w_o, B_x, B_w_r, B_w_gate, B_w_up, B_w_down):
    def _A_ref(x, c_kv, w_q, w_uk, w_uv, w_o):
        B, Sq, M = x.shape[0], x.shape[1], x.shape[2]
        Sk = c_kv.shape[1]
        H, D = w_q.shape[1], w_q.shape[2]
        q = jnp.einsum("bqm,mhd->bhqd", x, w_q)
        k = jnp.einsum("bkc,chd->bhkd", c_kv, w_uk)
        v = jnp.einsum("bkc,chd->bhkd", c_kv, w_uv)
        scores = jnp.einsum("bhqd,bhkd->bhqk", q, k) * (D ** -0.5)
        off = Sk - Sq
        qi = jnp.arange(Sq)[:, None]
        kj = jnp.arange(Sk)[None, :]
        cmask = kj <= (qi + off)
        scores = jnp.where(cmask[None, None], scores, -1e9)
        p = _softmax(scores, axis=-1)
        ctx = jnp.einsum("bhqk,bhkd->bhqd", p, v)
        return jnp.einsum("bhqd,hdm->bqm", ctx, w_o)

    def _B_ref(x, w_r, w_gate, w_up, w_down):
        B, S, D = x.shape
        C = 1
        r = x @ w_r
        idx = jnp.argsort(-r, axis=-1)[:, :C]
        idx_e = jnp.repeat(idx.reshape(B, C, 1), D, axis=2)
        x_sel = jnp.take_along_axis(x, idx_e, axis=1)
        g = _silu(x_sel @ w_gate)
        u = x_sel @ w_up
        y = (g * u) @ w_down
        r_sel = _sigmoid(jnp.take_along_axis(r, idx, axis=1))
        y = y * r_sel.reshape(B, C, 1)
        b_off = (jnp.arange(B) * S).reshape(B, 1)
        flat_idx = (idx + b_off).reshape(B * C)
        zero = (x * 0.0).reshape(B * S, D)
        upd = _scatter_add(zero, flat_idx, y.reshape(B * C, D), axis=0)
        return x + upd.reshape(B, S, D)

    x = A_x
    xn = _layernorm(x, axis=-1)
    s = _A_ref(xn, A_c_kv, A_w_q, A_w_uk, A_w_uv, A_w_o)
    g = _silu(_B_ref(xn, B_w_r, B_w_gate, B_w_up, B_w_down))
    return x + s * g
```

```python
import jax
import jax.numpy as jnp
from jax import lax
import jax.experimental.pallas as pl
import jax.experimental.pallas.tpu as pltpu

_F32 = jnp.float32
_BF16 = jnp.bfloat16
_HG = 16
_LANES = 128
_WO_HEADS = (17, 11, 3, 1)


def _dot(a, b):
    return jnp.dot(a, b, preferred_element_type=_F32)


def _dot_nt(a, b):
    return lax.dot_general(a, b, (((1,), (1,)), ((), ())), preferred_element_type=_F32)


def _iota(shape, axis):
    return lax.broadcasted_iota(jnp.int32, shape, axis)


def _sigmoid(v):
    return 1.0 / (1.0 + jnp.exp(-v))


def _kernel(
    x_hbm, ckv_hbm, wq_hbm, wuk_hbm, wuv_hbm, wo_hbm, wr_hbm, wg_hbm, wu_hbm, wd_hbm,
    out_hbm,
    x_v, ckv_v, wq_v, wuk_v, wuv_v, wr_v, wg_v, wu_v, wd_v, out_v, ctx_v, sems, *wo_vs,
):
    B, M = x_v.shape
    _, H, D = wq_v.shape
    Dc = wuk_v.shape[0]
    n_groups = H // _HG
    rows = B * _HG

    pairs = [
        (wq_hbm, wq_v), (x_hbm, x_v), (wr_hbm, wr_v), (wuk_hbm, wuk_v), (ckv_hbm, ckv_v),
        (wuv_hbm, wuv_v), (wg_hbm, wg_v), (wu_hbm, wu_v), (wd_hbm, wd_v),
    ]
    h0 = 0
    for wo_v in wo_vs:
        n = wo_v.shape[0]
        pairs.append((wo_hbm.at[pl.ds(h0, n)], wo_v))
        h0 += n
    copies = [pltpu.make_async_copy(s, d, sems.at[i]) for i, (s, d) in enumerate(pairs)]
    for cp in copies:
        cp.start()
    wq_cp, x_cp, wr_cp, wuk_cp, ckv_cp, wuv_cp, wg_cp, wu_cp, wd_cp, *wo_cps = copies

    wide = _LANES * _HG
    expand = (_iota((_LANES, wide), 1) // _HG == _iota((_LANES, wide), 0)).astype(_BF16)
    own_head = _iota((rows, wide), 1) % _HG == _iota((rows, wide), 0) % _HG

    wq_cp.wait()
    x_cp.wait()
    x = x_v[...].astype(_F32)
    mean = jnp.mean(x, axis=-1, keepdims=True)
    xc = x - mean
    var = jnp.mean(xc * xc, axis=-1, keepdims=True)
    xn_lo = (xc / jnp.sqrt(var + 1e-5)).astype(_BF16)
    xn = xn_lo.astype(_F32)

    xn_rows = jnp.concatenate(
        [jnp.broadcast_to(xn[b:b + 1], (_HG, M)) for b in range(B)], axis=0
    ).astype(_BF16)
    q = [jnp.zeros((rows, D), _F32) for _ in range(n_groups)]
    for m0 in range(0, M, _LANES):
        n = min(_LANES, M - m0)
        lhs = _dot(xn_rows[:, m0:m0 + n], expand[:n, :n * _HG])
        lhs = jnp.where(own_head[:, :n * _HG], lhs, 0.0).astype(_BF16)
        for g in range(n_groups):
            w = wq_v[m0:m0 + n, g * _HG:(g + 1) * _HG, :].reshape(n * _HG, D)
            q[g] = q[g] + _dot(lhs, w)

    wuk_cp.wait()
    q_lat = []
    for g in range(n_groups):
        qg = q[g].astype(_BF16)
        slabs = []
        for c0 in range(0, Dc, _LANES):
            w = wuk_v[c0:c0 + _LANES, g * _HG:(g + 1) * _HG, :].reshape(wide, D)
            full = jnp.where(own_head, _dot_nt(qg, w), 0.0).astype(_BF16)
            slabs.append(_dot_nt(full, expand))
        q_lat.append(jnp.concatenate(slabs, axis=1).astype(_BF16))

    ckv_cp.wait()
    lat = []
    for b in range(B):
        qb = jnp.concatenate([ql[b * _HG:(b + 1) * _HG] for ql in q_lat], axis=0)
        s = _dot_nt(qb, ckv_v[b]) * (D ** -0.5)
        p = jnp.exp(s - jnp.max(s, axis=-1, keepdims=True))
        denom = jnp.sum(p, axis=-1, keepdims=True)
        lat.append((_dot(p.astype(_BF16), ckv_v[b]) / denom).astype(_BF16))

    wuv_cp.wait()
    for g in range(n_groups):
        lg = jnp.concatenate([lb[g * _HG:(g + 1) * _HG] for lb in lat], axis=0)
        ctx = jnp.zeros((rows, D), _F32)
        for c0 in range(0, Dc, _LANES):
            lhs = _dot(lg[:, c0:c0 + _LANES], expand)
            lhs = jnp.where(own_head, lhs, 0.0).astype(_BF16)
            w = wuv_v[c0:c0 + _LANES, g * _HG:(g + 1) * _HG, :].reshape(wide, D)
            ctx = ctx + _dot(lhs, w)
        ctx_v[g * rows:(g + 1) * rows, :] = ctx

    wr_cp.wait()
    wr = wr_v[...].astype(_F32).reshape(1, M)
    route = _sigmoid(jnp.sum(xn * wr, axis=-1, keepdims=True))
    wg_cp.wait()
    gate = _dot(xn_lo, wg_v[...])
    gate = gate * _sigmoid(gate)
    wu_cp.wait()
    hidden = (gate * _dot(xn_lo, wu_v[...])).astype(_BF16)
    wd_cp.wait()
    t = xn + (xn * 0.0 + _dot_nt(hidden, wd_v[...]) * route)
    mix = t * _sigmoid(t)

    s = jnp.zeros((B, M), _F32)
    h = 0
    for wo_cp, wo_v in zip(wo_cps, wo_vs):
        wo_cp.wait()
        for i in range(wo_v.shape[0]):
            first = (h // _HG) * rows + h % _HG
            ch = ctx_v[pl.ds(first, B, stride=_HG), :].astype(_BF16)
            s = s + _dot_nt(ch, wo_v[i])
            h += 1

    out_v[...] = (x + s * mix).astype(out_v.dtype)
    out_cp = pltpu.make_async_copy(out_v, out_hbm, sems.at[len(copies)])
    out_cp.start()
    out_cp.wait()


@jax.jit
def pallas_recurrent_scan__compressed_kv_cla__moe_arch_mod__decode_kernel(
    A_x: jax.Array,
    A_c_kv: jax.Array,
    A_w_q: jax.Array,
    A_w_uk: jax.Array,
    A_w_uv: jax.Array,
    A_w_o: jax.Array,
    B_x: jax.Array,
    B_w_r: jax.Array,
    B_w_gate: jax.Array,
    B_w_up: jax.Array,
    B_w_down: jax.Array,
):
    del B_x
    B, Sq, M = A_x.shape
    _, H, D = A_w_q.shape
    assert Sq == 1 and H % _HG == 0 and sum(_WO_HEADS) == H

    x = A_x.reshape(B, M)
    w_o = jnp.transpose(A_w_o, (0, 2, 1))
    w_down = B_w_down.T

    def vmem(a):
        return pltpu.VMEM(a.shape, a.dtype)

    hbm = pl.BlockSpec(memory_space=pltpu.HBM)
    out = pl.pallas_call(
        _kernel,
        out_shape=jax.ShapeDtypeStruct((B, M), A_x.dtype),
        in_specs=[hbm] * 10,
        out_specs=hbm,
        scratch_shapes=[
            vmem(x), vmem(A_c_kv), vmem(A_w_q), vmem(A_w_uk), vmem(A_w_uv), vmem(B_w_r),
            vmem(B_w_gate), vmem(B_w_up), vmem(w_down), vmem(x),
            pltpu.VMEM((B * H, D), _F32),
            pltpu.SemaphoreType.DMA((10 + len(_WO_HEADS),)),
            *[pltpu.VMEM((n, M, D), w_o.dtype) for n in _WO_HEADS],
        ],
        compiler_params=pltpu.CompilerParams(vmem_limit_bytes=100 * 1024 * 1024),
    )(x, A_c_kv, A_w_q, A_w_uk, A_w_uv, w_o, B_w_r, B_w_gate, B_w_up, w_down)
    return out.reshape(B, Sq, M)
```

```python
import math

import jax
import jax.numpy as jnp
from jax import lax
import jax.experimental.pallas as pl
import jax.experimental.pallas.tpu as pltpu

_F32 = jnp.float32
_BF16 = jnp.bfloat16
_LANES = 128
_TILE_ROWS = 8
_SLAB = 32
_HG = 16

_PAGE = 4
_PAGE_START = 2
_LOW_PER_HIGH = 3
_LEAD = 24
_QUEUE = 88
_WO_GROUPS = (48, 20, 8, 4, 4)
_WO_FIRST_PAGE = 8


def _dot(a, b):
    return jnp.dot(a, b, preferred_element_type=_F32)


def _dot_nt(a, b):
    return lax.dot_general(a, b, (((1,), (1,)), ((), ())), preferred_element_type=_F32)


def _iota(shape, axis):
    return lax.broadcasted_iota(jnp.int32, shape, axis)


def _sigmoid(v):
    return 1.0 / (1.0 + jnp.exp(-v))


def _pad_rows(v):
    return jnp.concatenate([v, jnp.zeros((8 - v.shape[0], v.shape[1]), v.dtype)], axis=0)


def _pages(lo, hi, streams, first=0):
    start = lo + (_PAGE_START - lo) % _PAGE
    whole = list(range(start, hi - _PAGE + 1, _PAGE))
    step = -(-len(whole) // streams)
    while math.gcd(step, len(whole)) != 1:
        step += 1
    end = whole[-1] + _PAGE
    ragged = [(a, b - a) for a, b in ((end, hi), (lo, start)) if b > a]
    return ragged + [
        (whole[(first + i * step) % len(whole)], _PAGE) for i in range(len(whole))
    ]


class _Stream:
    def __init__(self, groups, buf, sems, n_low_at_end):
        self.groups, self.buf, self.sems = groups, buf, sems
        order = [(g, page) for g, (_, _, pages) in enumerate(groups) for page in pages]
        is_high = [
            i % (_LOW_PER_HIGH + 1) == 0 and i < len(order) - n_low_at_end
            for i in range(len(order))
        ]
        high = [c + (0,) for c, h in zip(order, is_high) if h]
        low = [c + (1,) for c, h in zip(order, is_high) if not h]
        self.todo, low = low[:_LEAD], low[_LEAD:]
        for i, c in enumerate(high):
            self.todo += [c] + low[i * _LOW_PER_HIGH:(i + 1) * _LOW_PER_HIGH]
        self.todo += low[len(high) * _LOW_PER_HIGH:]
        self.last = {g: i for i, (g, _, _) in enumerate(self.todo)}
        self.done = 0

    def advance(self, count=_LOW_PER_HIGH + 1):
        for g, (start, size), priority in self.todo[self.done:self.done + count]:
            src, base, _ = self.groups[g]
            pltpu.make_async_copy(
                src.at[pl.ds(start, size)],
                self.buf.at[pl.ds(base + start, size)],
                self.sems.at[g],
            ).start(priority=priority)
        self.done = min(self.done + count, len(self.todo))

    def wait(self, g):
        self.advance(max(self.last[g] + 1 + _QUEUE - self.done, 0))
        total = self.buf.at[pl.ds(0, sum(size for _, size in self.groups[g][2]))]
        pltpu.make_async_copy(total, total, self.sems.at[g]).wait()


def _kernel(
    x_hbm, wr_hbm, wq_hbm, wuk_hbm, ckv_hbm, wuv_hbm, wg_hbm, wu_hbm, wd_hbm, wo_hbm,
    out_hbm,
    buf, x_v, wr_v, out_v, ctx_v, sems, small_sems,
    *, heads, keys, hidden_dim,
):
    B, M = x_v.shape
    D = _LANES
    Dc = wuk_hbm.shape[0]
    n_groups = heads // _HG
    rows = B * _HG
    per_tile = _LANES // _HG
    n_expand = _LANES // per_tile

    sources = [wq_hbm, wuk_hbm, ckv_hbm, wuv_hbm, wg_hbm, wu_hbm, wd_hbm, wo_hbm]
    bases = [0]
    for src in sources:
        bases.append(bases[-1] + src.shape[0])
    q0, uk0, kv0, uv0, g0, u0, d0, o0, expand0 = bases
    lhs0 = expand0 + n_expand * _LANES // _SLAB

    def whole(src, base):
        return src, base, _pages(0, src.shape[0], streams=8)

    half = ckv_hbm.shape[0] // 2
    groups = [
        whole(wq_hbm, q0),
        whole(wuk_hbm, uk0),
        (ckv_hbm, kv0, _pages(0, half, streams=8)),
        (ckv_hbm, kv0, _pages(half, 2 * half, streams=8)),
        whole(wuv_hbm, uv0),
        whole(wg_hbm, g0),
        whole(wu_hbm, u0),
        whole(wd_hbm, d0),
    ]
    wo_pages = _pages(0, wo_hbm.shape[0], streams=8, first=_WO_FIRST_PAGE)
    cuts = [len(wo_pages) - sum(_WO_GROUPS[i:]) for i in range(len(_WO_GROUPS) + 1)]
    first_wo = len(groups)
    groups += [(wo_hbm, o0, wo_pages[a:b]) for a, b in zip([0] + cuts[:-1], cuts)]
    stream = _Stream(groups, buf, sems, n_low_at_end=sum(_WO_GROUPS[1:]))

    def flat(start, n):
        return buf[start:start + n].reshape(n * _SLAB, _LANES)

    def head_group(base, row0, n, g):
        return buf[base + row0:base + row0 + n, g * _HG:(g + 1) * _HG, :].reshape(n * _HG, D)

    def column_tile(base, width, row0, n, j):
        per_band = width // _LANES * _TILE_ROWS // _SLAB
        slab, row = divmod(j * _TILE_ROWS, _SLAB)
        first = base + row0 // _TILE_ROWS * per_band + slab
        bands = pl.ds(first, n // _TILE_ROWS, stride=per_band)
        return buf[bands, row:row + _TILE_ROWS, :].reshape(n, _LANES)

    def expand(t):
        return flat(expand0 + t * _LANES // _SLAB, _LANES // _SLAB)

    x_cp = pltpu.make_async_copy(x_hbm, x_v, small_sems.at[0])
    wr_cp = pltpu.make_async_copy(wr_hbm, wr_v, small_sems.at[1])
    stream.advance(_LEAD // 2)
    x_cp.start()
    wr_cp.start()
    stream.advance(_QUEUE)

    square = (_LANES, _LANES)
    for t in range(n_expand):
        e = _iota(square, 1) // _HG + t * per_tile == _iota(square, 0)
        first = expand0 + t * _LANES // _SLAB
        buf[first:first + _LANES // _SLAB] = e.astype(_BF16).reshape(-1, _SLAB, _LANES)
        if t % 4 == 3:
            stream.advance()
    own_head = _iota((rows, _LANES), 1) % _HG == _iota((rows, _LANES), 0) % _HG

    x_cp.wait()
    wr_cp.wait()
    x = _pad_rows(x_v[...].astype(_F32))
    xc = x - jnp.mean(x, axis=-1, keepdims=True)
    xn_lo = (xc / jnp.sqrt(jnp.mean(xc * xc, axis=-1, keepdims=True) + 1e-5)).astype(_BF16)
    xn = xn_lo.astype(_F32)
    wr = wr_v[...].astype(_F32).reshape(1, M)
    route = _sigmoid(jnp.sum(xn * wr, axis=-1, keepdims=True))

    lhs_slabs = rows // _SLAB
    for t in range(M // per_tile):
        m0 = t // n_expand * _LANES
        n = min(_LANES, M - m0)
        rep = _dot(xn_lo[:, m0:m0 + n], expand(t % n_expand)[:n])
        rep = jnp.concatenate(
            [jnp.broadcast_to(rep[b:b + 1], (_HG, _LANES)) for b in range(B)], axis=0
        )
        first = lhs0 + t * lhs_slabs
        buf[first:first + lhs_slabs] = (
            jnp.where(own_head, rep, 0.0).astype(_BF16).reshape(lhs_slabs, _SLAB, _LANES)
        )
        if t % 8 == 7:
            stream.advance()
    stream.wait(0)
    q = [jnp.zeros((rows, D), _F32) for _ in range(n_groups)]
    for t in range(M // per_tile):
        lhs = flat(lhs0 + t * lhs_slabs, lhs_slabs)
        for g in range(n_groups):
            q[g] = q[g] + _dot(lhs, head_group(q0, t * per_tile, per_tile, g))
        if t % 6 == 5:
            stream.advance()

    stream.wait(1)
    q_lat = []
    for g in range(n_groups):
        qg = q[g].astype(_BF16)
        tiles = []
        for c0 in range(0, Dc, _LANES):
            acc = jnp.zeros((rows, _LANES), _F32)
            for t in range(n_expand):
                full = _dot_nt(qg, head_group(uk0, c0 + t * per_tile, per_tile, g))
                acc = acc + _dot_nt(jnp.where(own_head, full, 0.0).astype(_BF16), expand(t))
                if t % 8 == 7:
                    stream.advance()
            tiles.append(acc.astype(_BF16))
        q_lat.append(tiles)

    qk_keys, pv_keys = 512, 1024
    lat = []
    for b in range(B):
        if b % (B // 2) == 0:
            stream.wait(2 + b // (B // 2))
        qb = [
            jnp.concatenate([q_lat[g][j][b * _HG:(b + 1) * _HG] for g in range(n_groups)], axis=0)
            for j in range(Dc // _LANES)
        ]
        scores = []
        for k0 in range(b * keys, (b + 1) * keys, qk_keys):
            parts = [
                _dot_nt(qj, column_tile(kv0, Dc, k0, qk_keys, j)) for j, qj in enumerate(qb)
            ]
            scores.append(sum(parts[1:], parts[0]))
            stream.advance()
        s = jnp.concatenate(scores, axis=1) * (D ** -0.5)
        p = jnp.exp(s - jnp.max(s, axis=-1, keepdims=True))
        denom = jnp.sum(p, axis=-1, keepdims=True)
        p = p.astype(_BF16)
        acc = [jnp.zeros((heads, _LANES), _F32) for _ in qb]
        for k0 in range(0, keys, pv_keys):
            stream.advance()
            acc = [
                a + _dot(p[:, k0:k0 + pv_keys], column_tile(kv0, Dc, b * keys + k0, pv_keys, j))
                for j, a in enumerate(acc)
            ]
        lat.append([(a / denom).astype(_BF16) for a in acc])

    stream.wait(4)
    for g in range(n_groups):
        ctx = jnp.zeros((rows, D), _F32)
        for j in range(Dc // _LANES):
            lg = jnp.concatenate([lb[j][g * _HG:(g + 1) * _HG] for lb in lat], axis=0)
            for t in range(n_expand):
                lhs = jnp.where(own_head, _dot(lg, expand(t)), 0.0).astype(_BF16)
                ctx = ctx + _dot(lhs, head_group(uv0, j * _LANES + t * per_tile, per_tile, g))
                if t % 8 == 7:
                    stream.advance()
        ctx_v[g * rows:(g + 1) * rows, :] = ctx

    def project(base):
        tiles = []
        for j in range(hidden_dim // _LANES):
            tiles.append(_dot(xn_lo, column_tile(base, hidden_dim, 0, M, j)))
            if j % 6 == 5:
                stream.advance()
        return tiles

    stream.wait(5)
    gate = [v * _sigmoid(v) for v in project(g0)]
    stream.wait(6)
    hidden = [(a * v).astype(_BF16) for a, v in zip(gate, project(u0))]
    stream.wait(7)
    y = jnp.zeros(x.shape, _F32)
    for j, hj in enumerate(hidden):
        y = y + _dot_nt(hj, column_tile(d0, hidden_dim, 0, M, j))
        if j % 3 == 2:
            stream.advance()
    mixed = xn + (xn * 0.0 + y * route)
    mixed = mixed * _sigmoid(mixed)

    def ctx_rows(h):
        first = h // _HG * rows + h % _HG
        return _pad_rows(ctx_v[pl.ds(first, B, stride=_HG), :]).astype(_BF16)

    def per_head(pages):
        for start, size in pages:
            while size:
                h, m_slab = divmod(start, M // _SLAB)
                n = min(size, M // _SLAB - m_slab)
                yield h, m_slab * _SLAB, start, n
                start, size = start + n, size - n

    def place(v, m0):
        pads = [jnp.zeros((v.shape[0], w), v.dtype) for w in (m0, M - m0 - v.shape[1])]
        return jnp.concatenate([a for a in (pads[0], v, pads[1]) if a.shape[1]], axis=1)

    lane_tiles = [(m0, min(_LANES, M - m0)) for m0 in range(0, M, _LANES)]
    s = {tile: jnp.zeros((x.shape[0], tile[1]), _F32) for tile in lane_tiles}
    for g in range(first_wo, len(groups)):
        work = list(per_head(groups[g][2]))
        lhs = {h: ctx_rows(h) for h in sorted({h for h, _, _, _ in work})}
        stream.wait(g)
        shifted = {}
        for h, m0, start, n in work:
            tile = (m0, n * _SLAB)
            into = s if tile in s else shifted
            part = _dot_nt(lhs[h], flat(o0 + start, n))
            into[tile] = into[tile] + part if tile in into else part
        for (m0, _), v in shifted.items():
            wide = place(v, m0)
            s = {(a, w): acc + wide[:, a:a + w] for (a, w), acc in s.items()}

    out = x + jnp.concatenate([s[tile] for tile in lane_tiles], axis=1) * mixed
    out_v[...] = out.astype(out_v.dtype)[:B]
    out_cp = pltpu.make_async_copy(out_v, out_hbm, small_sems.at[0])
    out_cp.start()
    out_cp.wait()


def _slabs(w):
    r, c = w.shape
    w = w.reshape(r // _TILE_ROWS, _TILE_ROWS, c // _LANES, _LANES)
    return w.transpose(0, 2, 1, 3).reshape(-1, _SLAB, _LANES)


@jax.jit
def pallas_recurrent_scan__compressed_kv_cla__moe_arch_mod__decode_kernel(
    A_x: jax.Array,
    A_c_kv: jax.Array,
    A_w_q: jax.Array,
    A_w_uk: jax.Array,
    A_w_uv: jax.Array,
    A_w_o: jax.Array,
    B_x: jax.Array,
    B_w_r: jax.Array,
    B_w_gate: jax.Array,
    B_w_up: jax.Array,
    B_w_down: jax.Array,
):
    del B_x
    B, Sq, M = A_x.shape
    _, Sk, Dc = A_c_kv.shape
    _, H, D = A_w_q.shape
    assert Sq == 1 and H == _SLAB and D == _LANES

    x = A_x.reshape(B, M)
    streamed = [
        A_w_q,
        A_w_uk,
        _slabs(A_c_kv.reshape(B * Sk, Dc)),
        A_w_uv,
        _slabs(B_w_gate),
        _slabs(B_w_up),
        _slabs(B_w_down.T),
        jnp.transpose(A_w_o, (0, 2, 1)).reshape(-1, _SLAB, _LANES),
    ]
    n_slabs = sum(w.shape[0] for w in streamed) + (_HG * _LANES + M * B * _HG * _HG // D) // _SLAB

    def kernel(*refs):
        _kernel(*refs, heads=H, keys=Sk, hidden_dim=B_w_gate.shape[1])

    hbm = pl.BlockSpec(memory_space=pltpu.HBM)
    out = pl.pallas_call(
        kernel,
        out_shape=jax.ShapeDtypeStruct((B, M), A_x.dtype),
        in_specs=[hbm] * (2 + len(streamed)),
        out_specs=hbm,
        scratch_shapes=[
            pltpu.VMEM((n_slabs, _SLAB, _LANES), _BF16),
            pltpu.VMEM(x.shape, x.dtype),
            pltpu.VMEM(B_w_r.shape, B_w_r.dtype),
            pltpu.VMEM(x.shape, x.dtype),
            pltpu.VMEM((B * H, D), _F32),
            pltpu.SemaphoreType.DMA((len(streamed) + 1 + len(_WO_GROUPS),)),
            pltpu.SemaphoreType.DMA((2,)),
        ],
        compiler_params=pltpu.CompilerParams(
            vmem_limit_bytes=96 * 1024 * 1024, disable_semaphore_checks=True
        ),
    )(x, B_w_r, *streamed)
    return out.reshape(B, Sq, M)
```

```python
import jax
import jax.numpy as jnp
from jax import lax
import jax.experimental.pallas as pl
import jax.experimental.pallas.tpu as pltpu

_F32 = jnp.float32
_BF16 = jnp.bfloat16
_LANES = 128
_TILE_ROWS = 8
_SLAB = 32
_HG = 16

_PAGE = 4
_PAGE_START = 2
_SPACING = 16
_CACHE_SPACING = 32
_LOW_PER_HIGH = 3
_LEAD = 26
_STEP = 5
_QUEUE = 82
_WO_GROUPS = (48, 20, 8, 4, 4)


def _dot(a, b):
    return jnp.dot(a, b, preferred_element_type=_F32)


def _dot_nt(a, b):
    return lax.dot_general(a, b, (((1,), (1,)), ((), ())), preferred_element_type=_F32)


def _iota(shape, axis):
    return lax.broadcasted_iota(jnp.int32, shape, axis)


def _sigmoid(v):
    return 1.0 / (1.0 + jnp.exp(-v))


def _pad_rows(v):
    return jnp.concatenate([v, jnp.zeros((8 - v.shape[0], v.shape[1]), v.dtype)], axis=0)


def _pages(n_slabs, spacing):
    whole = list(range(_PAGE_START, n_slabs - _PAGE + 1, _PAGE))
    ragged = [(whole[-1] + _PAGE, n_slabs), (0, _PAGE_START)]
    return [(a, b - a) for a, b in ragged if b > a] + [
        (start, _PAGE) for i in range(spacing) for start in whole[i::spacing]
    ]


class _Stream:
    def __init__(self, groups, buf, sems, n_low_at_end):
        self.groups, self.buf, self.sems = groups, buf, sems
        order = [(g, page) for g, (_, _, pages) in enumerate(groups) for page in pages]
        is_high = [
            i % (_LOW_PER_HIGH + 1) == 0 and i < len(order) - n_low_at_end
            for i in range(len(order))
        ]
        high = [c + (0,) for c, h in zip(order, is_high) if h]
        low = [c + (1,) for c, h in zip(order, is_high) if not h]
        self.todo, low = low[:_LEAD], low[_LEAD:]
        for i, c in enumerate(high):
            self.todo += [c] + low[i * _LOW_PER_HIGH:(i + 1) * _LOW_PER_HIGH]
        self.todo += low[len(high) * _LOW_PER_HIGH:]
        self.ready = {}
        for i, (g, _, priority) in enumerate(self.todo):
            self.ready[g] = max(self.ready.get(g, 0), i + (_QUEUE if priority else 8))
        self.done = 0

    def advance(self, count=None):
        count = _STEP if count is None else count
        for g, (start, size), priority in self.todo[self.done:self.done + count]:
            src, base, _ = self.groups[g]
            pltpu.make_async_copy(
                src.at[pl.ds(start, size)],
                self.buf.at[pl.ds(base + start, size)],
                self.sems.at[g],
            ).start(priority=priority)
        self.done = min(self.done + count, len(self.todo))

    def wait(self, g):
        self.advance(max(self.ready[g] - self.done, 0))
        total = self.buf.at[pl.ds(0, sum(size for _, size in self.groups[g][2]))]
        pltpu.make_async_copy(total, total, self.sems.at[g]).wait()


def _kernel(
    x_hbm, wr_hbm, wq_hbm, wuk_hbm, ckv_hbm, wuv_hbm, wg_hbm, wu_hbm, wd_hbm, wo_hbm,
    out_hbm,
    buf, x_v, wr_v, out_v, ctx_v, sems, small_sems,
    *, heads, keys, hidden_dim,
):
    B, M = x_v.shape
    D = _LANES
    Dc = wuk_hbm.shape[0]
    n_groups = heads // _HG
    rows = B * _HG
    per_tile = _LANES // _HG
    n_expand = _LANES // per_tile

    sources = [wq_hbm, wuk_hbm, ckv_hbm, wuv_hbm, wg_hbm, wu_hbm, wd_hbm, wo_hbm]
    bases = [0]
    for src in sources:
        bases.append(bases[-1] + src.shape[0])
    q0, uk0, kv0, uv0, g0, u0, d0, o0, expand0 = bases
    lhs0 = expand0 + n_expand * _LANES // _SLAB

    groups = [
        (src, base, _pages(src.shape[0], _CACHE_SPACING if src is ckv_hbm else _SPACING))
        for src, base in zip(sources, bases)
    ]
    first_wo = len(groups) - 1
    wo_pages = groups.pop()[2]
    n_last = sum(_WO_GROUPS[-3:])
    last = [
        (start, size) for start, size in wo_pages
        if size == _PAGE and start % (M // _SLAB) % _PAGE == 0
        and start % (M // _SLAB) + size <= M // _SLAB
    ][-n_last:]
    wo_pages = [page for page in wo_pages if page not in last] + last
    cuts = [len(wo_pages) - sum(_WO_GROUPS[i:]) for i in range(len(_WO_GROUPS) + 1)]
    groups += [(wo_hbm, o0, wo_pages[a:b]) for a, b in zip([0] + cuts[:-1], cuts)]
    stream = _Stream(groups, buf, sems, n_low_at_end=sum(_WO_GROUPS[1:]))

    def flat(start, n):
        return buf[start:start + n].reshape(n * _SLAB, _LANES)

    def head_group(base, row0, n, g):
        return buf[base + row0:base + row0 + n, g * _HG:(g + 1) * _HG, :].reshape(n * _HG, D)

    def column_tile(base, width, row0, n, j):
        per_band = width // _LANES * _TILE_ROWS // _SLAB
        slab, row = divmod(j * _TILE_ROWS, _SLAB)
        first = base + row0 // _TILE_ROWS * per_band + slab
        bands = pl.ds(first, n // _TILE_ROWS, stride=per_band)
        return buf[bands, row:row + _TILE_ROWS, :].reshape(n, _LANES)

    def expand(t):
        return flat(expand0 + t * _LANES // _SLAB, _LANES // _SLAB)

    x_cp = pltpu.make_async_copy(x_hbm, x_v, small_sems.at[0])
    wr_cp = pltpu.make_async_copy(wr_hbm, wr_v, small_sems.at[1])
    stream.advance(_LEAD // 2)
    x_cp.start()
    wr_cp.start()
    stream.advance(_QUEUE)

    square = (_LANES, _LANES)
    for t in range(n_expand):
        e = _iota(square, 1) // _HG + t * per_tile == _iota(square, 0)
        first = expand0 + t * _LANES // _SLAB
        buf[first:first + _LANES // _SLAB] = e.astype(_BF16).reshape(-1, _SLAB, _LANES)
        if t % 4 == 3:
            stream.advance()
    own_head = _iota((rows, _LANES), 1) % _HG == _iota((rows, _LANES), 0) % _HG

    x_cp.wait()
    wr_cp.wait()
    x = _pad_rows(x_v[...].astype(_F32))
    xc = x - jnp.mean(x, axis=-1, keepdims=True)
    xn_lo = (xc / jnp.sqrt(jnp.mean(xc * xc, axis=-1, keepdims=True) + 1e-5)).astype(_BF16)
    xn = xn_lo.astype(_F32)
    wr = wr_v[...].astype(_F32).reshape(1, M)
    route = _sigmoid(jnp.sum(xn * wr, axis=-1, keepdims=True))

    lhs_slabs = rows // _SLAB
    for t in range(M // per_tile):
        m0 = t // n_expand * _LANES
        n = min(_LANES, M - m0)
        rep = _dot(xn_lo[:, m0:m0 + n], expand(t % n_expand)[:n])
        rep = jnp.concatenate(
            [jnp.broadcast_to(rep[b:b + 1], (_HG, _LANES)) for b in range(B)], axis=0
        )
        first = lhs0 + t * lhs_slabs
        buf[first:first + lhs_slabs] = (
            jnp.where(own_head, rep, 0.0).astype(_BF16).reshape(lhs_slabs, _SLAB, _LANES)
        )
        if t % 8 == 7:
            stream.advance()
    stream.wait(0)
    q = [jnp.zeros((rows, D), _F32) for _ in range(n_groups)]
    for t in range(M // per_tile):
        lhs = flat(lhs0 + t * lhs_slabs, lhs_slabs)
        for g in range(n_groups):
            q[g] = q[g] + _dot(lhs, head_group(q0, t * per_tile, per_tile, g))
        if t % 6 == 5:
            stream.advance()

    stream.wait(1)
    q_lat = []
    for g in range(n_groups):
        qg = q[g].astype(_BF16)
        tiles = []
        for c0 in range(0, Dc, _LANES):
            acc = jnp.zeros((rows, _LANES), _F32)
            for t in range(n_expand):
                full = _dot_nt(qg, head_group(uk0, c0 + t * per_tile, per_tile, g))
                acc = acc + _dot_nt(jnp.where(own_head, full, 0.0).astype(_BF16), expand(t))
                if t % 8 == 7:
                    stream.advance()
            tiles.append(acc.astype(_BF16))
        q_lat.append(tiles)

    qk_keys, pv_keys = 512, 1024
    lat_tiles = range(Dc // _LANES)

    def scores(b):
        qb = [
            jnp.concatenate([q_lat[g][j][b * _HG:(b + 1) * _HG] for g in range(n_groups)], axis=0)
            for j in lat_tiles
        ]
        chunks = []
        for k0 in range(b * keys, (b + 1) * keys, qk_keys):
            parts = [_dot_nt(qb[j], column_tile(kv0, Dc, k0, qk_keys, j)) for j in lat_tiles]
            chunks.append(sum(parts[1:], parts[0]))
            stream.advance()
        return jnp.concatenate(chunks, axis=1) * (D ** -0.5)

    def attend(b, s):
        p = jnp.exp(s - jnp.max(s, axis=-1, keepdims=True))
        denom = jnp.sum(p, axis=-1, keepdims=True)
        p = p.astype(_BF16)
        acc = [jnp.zeros((heads, _LANES), _F32) for _ in lat_tiles]
        for k0 in range(0, keys, pv_keys):
            acc = [
                a + _dot(p[:, k0:k0 + pv_keys], column_tile(kv0, Dc, b * keys + k0, pv_keys, j))
                for j, a in enumerate(acc)
            ]
            stream.advance()
        return [(a / denom).astype(_BF16) for a in acc]

    stream.wait(2)
    lat = []
    s = scores(0)
    for b in range(B):
        ahead = scores(b + 1) if b + 1 < B else None
        lat.append(attend(b, s))
        s = ahead

    stream.wait(3)
    for g in range(n_groups):
        ctx = jnp.zeros((rows, D), _F32)
        for j in range(Dc // _LANES):
            lg = jnp.concatenate([lb[j][g * _HG:(g + 1) * _HG] for lb in lat], axis=0)
            for t in range(n_expand):
                lhs = jnp.where(own_head, _dot(lg, expand(t)), 0.0).astype(_BF16)
                ctx = ctx + _dot(lhs, head_group(uv0, j * _LANES + t * per_tile, per_tile, g))
                if t % 8 == 7:
                    stream.advance()
        ctx_v[g * rows:(g + 1) * rows, :] = ctx

    def project(base):
        tiles = []
        for j in range(hidden_dim // _LANES):
            tiles.append(_dot(xn_lo, column_tile(base, hidden_dim, 0, M, j)))
            if j % 6 == 5:
                stream.advance()
        return tiles

    stream.wait(4)
    gate = [v * _sigmoid(v) for v in project(g0)]
    stream.wait(5)
    hidden = [(a * v).astype(_BF16) for a, v in zip(gate, project(u0))]
    stream.wait(6)
    y = jnp.zeros(x.shape, _F32)
    for j, hj in enumerate(hidden):
        y = y + _dot_nt(hj, column_tile(d0, hidden_dim, 0, M, j))
        if j % 3 == 2:
            stream.advance()
    mixed = xn + (xn * 0.0 + y * route)
    mixed = mixed * _sigmoid(mixed)

    def ctx_rows(h):
        first = h // _HG * rows + h % _HG
        return _pad_rows(ctx_v[pl.ds(first, B, stride=_HG), :]).astype(_BF16)

    def per_head(pages):
        for start, size in pages:
            while size:
                h, m_slab = divmod(start, M // _SLAB)
                n = min(size, M // _SLAB - m_slab)
                yield h, m_slab * _SLAB, start, n
                start, size = start + n, size - n

    def place(v, m0):
        pads = [jnp.zeros((v.shape[0], w), v.dtype) for w in (m0, M - m0 - v.shape[1])]
        return jnp.concatenate([a for a in (pads[0], v, pads[1]) if a.shape[1]], axis=1)

    lane_tiles = [(m0, min(_LANES, M - m0)) for m0 in range(0, M, _LANES)]
    s = {tile: jnp.zeros((x.shape[0], tile[1]), _F32) for tile in lane_tiles}
    for g in range(first_wo, len(groups)):
        work = list(per_head(groups[g][2]))
        lhs = {h: ctx_rows(h) for h in sorted({h for h, _, _, _ in work})}
        stream.wait(g)
        shifted = {}
        for h, m0, start, n in work:
            tile = (m0, n * _SLAB)
            into = s if tile in s else shifted
            part = _dot_nt(lhs[h], flat(o0 + start, n))
            into[tile] = into[tile] + part if tile in into else part
        for (m0, _), v in shifted.items():
            wide = place(v, m0)
            s = {(a, w): acc + wide[:, a:a + w] for (a, w), acc in s.items()}

    out = x + jnp.concatenate([s[tile] for tile in lane_tiles], axis=1) * mixed
    out_v[...] = out.astype(out_v.dtype)[:B]
    out_cp = pltpu.make_async_copy(out_v, out_hbm, small_sems.at[0])
    out_cp.start()
    out_cp.wait()


def _slabs(w):
    r, c = w.shape
    w = w.reshape(r // _TILE_ROWS, _TILE_ROWS, c // _LANES, _LANES)
    return w.transpose(0, 2, 1, 3).reshape(-1, _SLAB, _LANES)


@jax.jit
def pallas_recurrent_scan__compressed_kv_cla__moe_arch_mod__decode_kernel(
    A_x: jax.Array,
    A_c_kv: jax.Array,
    A_w_q: jax.Array,
    A_w_uk: jax.Array,
    A_w_uv: jax.Array,
    A_w_o: jax.Array,
    B_x: jax.Array,
    B_w_r: jax.Array,
    B_w_gate: jax.Array,
    B_w_up: jax.Array,
    B_w_down: jax.Array,
):
    del B_x
    B, Sq, M = A_x.shape
    _, Sk, Dc = A_c_kv.shape
    _, H, D = A_w_q.shape
    assert Sq == 1 and H == _SLAB and D == _LANES

    x = A_x.reshape(B, M)
    streamed = [
        A_w_q,
        A_w_uk,
        _slabs(A_c_kv.reshape(B * Sk, Dc)),
        A_w_uv,
        _slabs(B_w_gate),
        _slabs(B_w_up),
        _slabs(B_w_down.T),
        jnp.transpose(A_w_o, (0, 2, 1)).reshape(-1, _SLAB, _LANES),
    ]
    n_slabs = sum(w.shape[0] for w in streamed) + (_HG * _LANES + M * B * _HG * _HG // D) // _SLAB

    def kernel(*refs):
        _kernel(*refs, heads=H, keys=Sk, hidden_dim=B_w_gate.shape[1])

    hbm = pl.BlockSpec(memory_space=pltpu.HBM)
    out = pl.pallas_call(
        kernel,
        out_shape=jax.ShapeDtypeStruct((B, M), A_x.dtype),
        in_specs=[hbm] * (2 + len(streamed)),
        out_specs=hbm,
        scratch_shapes=[
            pltpu.VMEM((n_slabs, _SLAB, _LANES), _BF16),
            pltpu.VMEM(x.shape, x.dtype),
            pltpu.VMEM(B_w_r.shape, B_w_r.dtype),
            pltpu.VMEM(x.shape, x.dtype),
            pltpu.VMEM((B * H, D), _F32),
            pltpu.SemaphoreType.DMA((len(streamed) + len(_WO_GROUPS),)),
            pltpu.SemaphoreType.DMA((2,)),
        ],
        compiler_params=pltpu.CompilerParams(
            vmem_limit_bytes=96 * 1024 * 1024, disable_semaphore_checks=True
        ),
    )(x, B_w_r, *streamed)
    return out.reshape(B, Sq, M)
```

```python
import jax
import jax.numpy as jnp
from jax import lax
import jax.experimental.pallas as pl
import jax.experimental.pallas.tpu as pltpu

_F32 = jnp.float32
_BF16 = jnp.bfloat16
_LANES = 128
_TILE_ROWS = 8
_SLAB = 32
_HG = 16

_PAGE = 4
_PAGE_START = 2
_SPACING = 16
_CACHE_SPACING = 32
_LOW_PER_HIGH = 3
_LEAD = 26
_STEP = 5
_LOW_AT_END = 20
_QUEUE = 82
_WO_GROUPS = (36, 12, 8, 4, 4, 4)


def _dot(a, b):
    return jnp.dot(a, b, preferred_element_type=_F32)


def _dot_nt(a, b):
    return lax.dot_general(a, b, (((1,), (1,)), ((), ())), preferred_element_type=_F32)


def _iota(shape, axis):
    return lax.broadcasted_iota(jnp.int32, shape, axis)


def _sigmoid(v):
    return 1.0 / (1.0 + jnp.exp(-v))


def _pad_rows(v):
    return jnp.concatenate([v, jnp.zeros((8 - v.shape[0], v.shape[1]), v.dtype)], axis=0)


def _pages(n_slabs, spacing):
    whole = list(range(_PAGE_START, n_slabs - _PAGE + 1, _PAGE))
    ragged = [(whole[-1] + _PAGE, n_slabs), (0, _PAGE_START)]
    return [(a, b - a) for a, b in ragged if b > a] + [
        (start, _PAGE) for i in range(spacing) for start in whole[i::spacing]
    ]


class _Stream:
    def __init__(self, groups, buf, sems, n_low_at_end):
        self.groups, self.buf, self.sems = groups, buf, sems
        order = [(g, page) for g, (_, _, pages) in enumerate(groups) for page in pages]
        is_high = [
            i % (_LOW_PER_HIGH + 1) == 0 and i < len(order) - n_low_at_end
            for i in range(len(order))
        ]
        high = [c + (0,) for c, h in zip(order, is_high) if h]
        low = [c + (1,) for c, h in zip(order, is_high) if not h]
        self.todo, low = low[:_LEAD], low[_LEAD:]
        for i, c in enumerate(high):
            self.todo += [c] + low[i * _LOW_PER_HIGH:(i + 1) * _LOW_PER_HIGH]
        self.todo += low[len(high) * _LOW_PER_HIGH:]
        self.ready = {}
        for i, (g, _, priority) in enumerate(self.todo):
            self.ready[g] = max(self.ready.get(g, 0), i + (_QUEUE if priority else 8))
        self.done = 0

    def advance(self, count=None):
        count = _STEP if count is None else count
        for g, (start, size), priority in self.todo[self.done:self.done + count]:
            src, base, _ = self.groups[g]
            pltpu.make_async_copy(
                src.at[pl.ds(start, size)],
                self.buf.at[pl.ds(base + start, size)],
                self.sems.at[g],
            ).start(priority=priority)
        self.done = min(self.done + count, len(self.todo))

    def wait(self, g):
        self.advance(max(self.ready[g] - self.done, 0))
        total = self.buf.at[pl.ds(0, sum(size for _, size in self.groups[g][2]))]
        pltpu.make_async_copy(total, total, self.sems.at[g]).wait()


def _kernel(
    x_hbm, wr_hbm, wq_hbm, wuk_hbm, ckv_hbm, wuv_hbm, wg_hbm, wu_hbm, wd_hbm, wo_hbm,
    out_hbm,
    buf, x_v, wr_v, out_v, ctx_v, sems, small_sems,
    *, heads, keys, hidden_dim,
):
    B, M = x_v.shape
    D = _LANES
    Dc = wuk_hbm.shape[0]
    n_groups = heads // _HG
    rows = B * _HG
    per_tile = _LANES // _HG
    n_expand = _LANES // per_tile

    sources = [wq_hbm, wuk_hbm, ckv_hbm, wuv_hbm, wg_hbm, wu_hbm, wd_hbm, wo_hbm]
    bases = [0]
    for src in sources:
        bases.append(bases[-1] + src.shape[0])
    q0, uk0, kv0, uv0, g0, u0, d0, o0, expand0 = bases
    lhs0 = expand0 + n_expand * _LANES // _SLAB

    groups = [
        (src, base, _pages(src.shape[0], _CACHE_SPACING if src is ckv_hbm else _SPACING))
        for src, base in zip(sources, bases)
    ]
    first_wo = len(groups) - 1
    wo_pages = groups.pop()[2]
    last = [
        (start, size) for start, size in wo_pages
        if size == _PAGE and start % (M // _SLAB) % _PAGE == 0
        and start % (M // _SLAB) + size <= M // _SLAB
    ][-_LOW_AT_END:]
    wo_pages = [page for page in wo_pages if page not in last] + last
    cuts = [len(wo_pages) - sum(_WO_GROUPS[i:]) for i in range(len(_WO_GROUPS) + 1)]
    groups += [(wo_hbm, o0, wo_pages[a:b]) for a, b in zip([0] + cuts[:-1], cuts)]
    stream = _Stream(groups, buf, sems, n_low_at_end=_LOW_AT_END)

    def flat(start, n):
        return buf[start:start + n].reshape(n * _SLAB, _LANES)

    def head_group(base, row0, n, g):
        return buf[base + row0:base + row0 + n, g * _HG:(g + 1) * _HG, :].reshape(n * _HG, D)

    def column_tile(base, width, row0, n, j):
        per_band = width // _LANES * _TILE_ROWS // _SLAB
        slab, row = divmod(j * _TILE_ROWS, _SLAB)
        first = base + row0 // _TILE_ROWS * per_band + slab
        bands = pl.ds(first, n // _TILE_ROWS, stride=per_band)
        return buf[bands, row:row + _TILE_ROWS, :].reshape(n, _LANES)

    def expand(t):
        return flat(expand0 + t * _LANES // _SLAB, _LANES // _SLAB)

    x_cp = pltpu.make_async_copy(x_hbm, x_v, small_sems.at[0])
    wr_cp = pltpu.make_async_copy(wr_hbm, wr_v, small_sems.at[1])
    stream.advance(_LEAD // 2)
    x_cp.start()
    wr_cp.start()
    stream.advance(_QUEUE)

    square = (_LANES, _LANES)
    for t in range(n_expand):
        e = _iota(square, 1) // _HG + t * per_tile == _iota(square, 0)
        first = expand0 + t * _LANES // _SLAB
        buf[first:first + _LANES // _SLAB] = e.astype(_BF16).reshape(-1, _SLAB, _LANES)
        if t % 4 == 3:
            stream.advance()
    own_head = _iota((rows, _LANES), 1) % _HG == _iota((rows, _LANES), 0) % _HG

    x_cp.wait()
    wr_cp.wait()
    x = _pad_rows(x_v[...].astype(_F32))
    xc = x - jnp.mean(x, axis=-1, keepdims=True)
    xn_lo = (xc / jnp.sqrt(jnp.mean(xc * xc, axis=-1, keepdims=True) + 1e-5)).astype(_BF16)
    xn = xn_lo.astype(_F32)
    wr = wr_v[...].astype(_F32).reshape(1, M)
    route = _sigmoid(jnp.sum(xn * wr, axis=-1, keepdims=True))

    lhs_slabs = rows // _SLAB
    for t in range(M // per_tile):
        m0 = t // n_expand * _LANES
        n = min(_LANES, M - m0)
        rep = _dot(xn_lo[:, m0:m0 + n], expand(t % n_expand)[:n])
        rep = jnp.concatenate(
            [jnp.broadcast_to(rep[b:b + 1], (_HG, _LANES)) for b in range(B)], axis=0
        )
        first = lhs0 + t * lhs_slabs
        buf[first:first + lhs_slabs] = (
            jnp.where(own_head, rep, 0.0).astype(_BF16).reshape(lhs_slabs, _SLAB, _LANES)
        )
        if t % 8 == 7:
            stream.advance()
    stream.wait(0)
    q = [jnp.zeros((rows, D), _F32) for _ in range(n_groups)]
    for t in range(M // per_tile):
        lhs = flat(lhs0 + t * lhs_slabs, lhs_slabs)
        for g in range(n_groups):
            q[g] = q[g] + _dot(lhs, head_group(q0, t * per_tile, per_tile, g))
        if t % 6 == 5:
            stream.advance()

    stream.wait(1)
    q_lat = []
    for g in range(n_groups):
        qg = q[g].astype(_BF16)
        tiles = []
        for c0 in range(0, Dc, _LANES):
            acc = jnp.zeros((rows, _LANES), _F32)
            for t in range(n_expand):
                full = _dot_nt(qg, head_group(uk0, c0 + t * per_tile, per_tile, g))
                acc = acc + _dot_nt(jnp.where(own_head, full, 0.0).astype(_BF16), expand(t))
                if t % 8 == 7:
                    stream.advance()
            tiles.append(acc.astype(_BF16))
        q_lat.append(tiles)

    qk_keys, pv_keys = 512, 1024
    lat_tiles = range(Dc // _LANES)

    def scores(b):
        qb = [
            jnp.concatenate([q_lat[g][j][b * _HG:(b + 1) * _HG] for g in range(n_groups)], axis=0)
            for j in lat_tiles
        ]
        chunks = []
        for k0 in range(b * keys, (b + 1) * keys, qk_keys):
            parts = [_dot_nt(qb[j], column_tile(kv0, Dc, k0, qk_keys, j)) for j in lat_tiles]
            chunks.append(sum(parts[1:], parts[0]))
            stream.advance()
        return jnp.concatenate(chunks, axis=1) * (D ** -0.5)

    def attend(b, s):
        p = jnp.exp(s - jnp.max(s, axis=-1, keepdims=True))
        denom = jnp.sum(p, axis=-1, keepdims=True)
        p = p.astype(_BF16)
        acc = [jnp.zeros((heads, _LANES), _F32) for _ in lat_tiles]
        for k0 in range(0, keys, pv_keys):
            acc = [
                a + _dot(p[:, k0:k0 + pv_keys], column_tile(kv0, Dc, b * keys + k0, pv_keys, j))
                for j, a in enumerate(acc)
            ]
            stream.advance()
        return [(a / denom).astype(_BF16) for a in acc]

    stream.wait(2)
    lat = []
    s = scores(0)
    for b in range(B):
        ahead = scores(b + 1) if b + 1 < B else None
        lat.append(attend(b, s))
        s = ahead

    stream.wait(3)
    for g in range(n_groups):
        ctx = jnp.zeros((rows, D), _F32)
        for j in range(Dc // _LANES):
            lg = jnp.concatenate([lb[j][g * _HG:(g + 1) * _HG] for lb in lat], axis=0)
            for t in range(n_expand):
                lhs = jnp.where(own_head, _dot(lg, expand(t)), 0.0).astype(_BF16)
                ctx = ctx + _dot(lhs, head_group(uv0, j * _LANES + t * per_tile, per_tile, g))
                if t % 8 == 7:
                    stream.advance()
        ctx_v[g * rows:(g + 1) * rows, :] = ctx

    def project(base):
        tiles = []
        for j in range(hidden_dim // _LANES):
            tiles.append(_dot(xn_lo, column_tile(base, hidden_dim, 0, M, j)))
            if j % 6 == 5:
                stream.advance()
        return tiles

    stream.wait(4)
    gate = [v * _sigmoid(v) for v in project(g0)]
    stream.wait(5)
    hidden = [(a * v).astype(_BF16) for a, v in zip(gate, project(u0))]
    stream.wait(6)
    y = jnp.zeros(x.shape, _F32)
    for j, hj in enumerate(hidden):
        y = y + _dot_nt(hj, column_tile(d0, hidden_dim, 0, M, j))
        if j % 3 == 2:
            stream.advance()
    mixed = xn + (xn * 0.0 + y * route)
    mixed = mixed * _sigmoid(mixed)

    def ctx_rows(h):
        first = h // _HG * rows + h % _HG
        return _pad_rows(ctx_v[pl.ds(first, B, stride=_HG), :]).astype(_BF16)

    def per_head(pages):
        for start, size in pages:
            while size:
                h, m_slab = divmod(start, M // _SLAB)
                n = min(size, M // _SLAB - m_slab)
                yield h, m_slab * _SLAB, start, n
                start, size = start + n, size - n

    def place(v, m0):
        pads = [jnp.zeros((v.shape[0], w), v.dtype) for w in (m0, M - m0 - v.shape[1])]
        return jnp.concatenate([a for a in (pads[0], v, pads[1]) if a.shape[1]], axis=1)

    lane_tiles = [(m0, min(_LANES, M - m0)) for m0 in range(0, M, _LANES)]
    s = {tile: jnp.zeros((x.shape[0], tile[1]), _F32) for tile in lane_tiles}
    shifted = {}
    for g in range(first_wo, len(groups)):
        work = list(per_head(groups[g][2]))
        lhs = {h: ctx_rows(h) for h in sorted({h for h, _, _, _ in work})}
        stream.wait(g)
        for (m0, _), v in shifted.items():
            wide = place(v, m0)
            s = {(a, w): acc + wide[:, a:a + w] for (a, w), acc in s.items()}
        shifted = {}
        for h, m0, start, n in work:
            tile = (m0, n * _SLAB)
            into = s if tile in s else shifted
            part = _dot_nt(lhs[h], flat(o0 + start, n))
            into[tile] = into[tile] + part if tile in into else part
    assert not shifted

    out = x + jnp.concatenate([s[tile] for tile in lane_tiles], axis=1) * mixed
    out_v[...] = out.astype(out_v.dtype)[:B]
    out_cp = pltpu.make_async_copy(out_v, out_hbm, small_sems.at[0])
    out_cp.start()
    out_cp.wait()


def _slabs(w):
    r, c = w.shape
    w = w.reshape(r // _TILE_ROWS, _TILE_ROWS, c // _LANES, _LANES)
    return w.transpose(0, 2, 1, 3).reshape(-1, _SLAB, _LANES)


@jax.jit
def pallas_recurrent_scan__compressed_kv_cla__moe_arch_mod__decode_kernel(
    A_x: jax.Array,
    A_c_kv: jax.Array,
    A_w_q: jax.Array,
    A_w_uk: jax.Array,
    A_w_uv: jax.Array,
    A_w_o: jax.Array,
    B_x: jax.Array,
    B_w_r: jax.Array,
    B_w_gate: jax.Array,
    B_w_up: jax.Array,
    B_w_down: jax.Array,
):
    del B_x
    B, Sq, M = A_x.shape
    _, Sk, Dc = A_c_kv.shape
    _, H, D = A_w_q.shape
    assert Sq == 1 and H == _SLAB and D == _LANES

    x = A_x.reshape(B, M)
    streamed = [
        A_w_q,
        A_w_uk,
        _slabs(A_c_kv.reshape(B * Sk, Dc)),
        A_w_uv,
        _slabs(B_w_gate),
        _slabs(B_w_up),
        _slabs(B_w_down.T),
        jnp.transpose(A_w_o, (0, 2, 1)).reshape(-1, _SLAB, _LANES),
    ]
    n_slabs = sum(w.shape[0] for w in streamed) + (_HG * _LANES + M * B * _HG * _HG // D) // _SLAB

    def kernel(*refs):
        _kernel(*refs, heads=H, keys=Sk, hidden_dim=B_w_gate.shape[1])

    hbm = pl.BlockSpec(memory_space=pltpu.HBM)
    out = pl.pallas_call(
        kernel,
        out_shape=jax.ShapeDtypeStruct((B, M), A_x.dtype),
        in_specs=[hbm] * (2 + len(streamed)),
        out_specs=hbm,
        scratch_shapes=[
            pltpu.VMEM((n_slabs, _SLAB, _LANES), _BF16),
            pltpu.VMEM(x.shape, x.dtype),
            pltpu.VMEM(B_w_r.shape, B_w_r.dtype),
            pltpu.VMEM(x.shape, x.dtype),
            pltpu.VMEM((B * H, D), _F32),
            pltpu.SemaphoreType.DMA((len(streamed) + len(_WO_GROUPS),)),
            pltpu.SemaphoreType.DMA((2,)),
        ],
        compiler_params=pltpu.CompilerParams(
            vmem_limit_bytes=96 * 1024 * 1024, disable_semaphore_checks=True
        ),
    )(x, B_w_r, *streamed)
    return out.reshape(B, Sq, M)
```

```python
import jax
import jax.numpy as jnp
from jax import lax
import jax.experimental.pallas as pl
import jax.experimental.pallas.tpu as pltpu

_F32 = jnp.float32
_BF16 = jnp.bfloat16
_LANES = 128
_TILE_ROWS = 8
_SLAB = 32
_HG = 16

_PAGE = 4
_PAGE_START = 2
_SPACING = 16
_CACHE_SPACING = 32
_LOW_PER_HIGH = 3
_LEAD = 26
_STEP = 5
_LOW_AT_END = 20
_QUEUE = 82
_WO_GROUPS = (36, 12, 8, 4, 4, 4)


def _dot(a, b):
    return jnp.dot(a, b, preferred_element_type=_F32)


def _dot_nt(a, b):
    return lax.dot_general(a, b, (((1,), (1,)), ((), ())), preferred_element_type=_F32)


def _iota(shape, axis):
    return lax.broadcasted_iota(jnp.int32, shape, axis)


def _pad_rows(v):
    return jnp.concatenate([v, jnp.zeros((8 - v.shape[0], v.shape[1]), v.dtype)], axis=0)


def _pages(n_slabs, spacing):
    whole = list(range(_PAGE_START, n_slabs - _PAGE + 1, _PAGE))
    ragged = [(whole[-1] + _PAGE, n_slabs), (0, _PAGE_START)]
    return [(a, b - a) for a, b in ragged if b > a] + [
        (start, _PAGE) for i in range(spacing) for start in whole[i::spacing]
    ]


class _Stream:
    def __init__(self, groups, buf, sems):
        self.groups, self.buf, self.sems = groups, buf, sems
        order = [(g, page) for g, (_, _, pages) in enumerate(groups) for page in pages]
        is_high = [
            i % (_LOW_PER_HIGH + 1) == 0 and i < len(order) - _LOW_AT_END
            for i in range(len(order))
        ]
        high = [c + (0,) for c, h in zip(order, is_high) if h]
        low = [c + (1,) for c, h in zip(order, is_high) if not h]
        self.todo, low = low[:_LEAD], low[_LEAD:]
        for i, c in enumerate(high):
            self.todo += [c] + low[i * _LOW_PER_HIGH:(i + 1) * _LOW_PER_HIGH]
        self.todo += low[len(high) * _LOW_PER_HIGH:]
        self.ready = {}
        for i, (g, _, priority) in enumerate(self.todo):
            self.ready[g] = max(self.ready.get(g, 0), i + (_QUEUE if priority else 8))
        self.done = 0

    def _copy(self, g, page):
        src, base, _ = self.groups[g]
        start, size = page
        return pltpu.make_async_copy(
            src.at[pl.ds(start, size)], self.buf.at[pl.ds(base + start, size)], self.sems.at[g]
        )

    def advance(self, count=None):
        count = _STEP if count is None else count
        for g, page, priority in self.todo[self.done:self.done + count]:
            self._copy(g, page).start(priority=priority)
        self.done = min(self.done + count, len(self.todo))

    def wait(self, g):
        self.advance(max(self.ready[g] - self.done, 0))
        src, base, pages = self.groups[g]
        if sum(size for _, size in pages) == src.shape[0]:
            filled = self.buf.at[pl.ds(base, src.shape[0])]
            pltpu.make_async_copy(filled, filled, self.sems.at[g]).wait()
        else:
            for page in pages:
                self._copy(g, page).wait()


def _kernel(
    x_hbm, wr_hbm, wq_hbm, wuk_hbm, ckv_hbm, wuv_hbm, wg_hbm, wu_hbm, wd_hbm, wo_hbm,
    out_hbm,
    buf, x_v, wr_v, out_v, ctx_v, sems, small_sems,
    *, heads, keys, hidden_dim,
):
    B, M = x_v.shape
    D = _LANES
    Dc = wuk_hbm.shape[0]
    n_groups = heads // _HG
    rows = B * _HG
    per_tile = _LANES // _HG
    n_expand = _LANES // per_tile

    sources = [wq_hbm, wuk_hbm, ckv_hbm, wuv_hbm, wg_hbm, wu_hbm, wd_hbm, wo_hbm]
    bases = [0]
    for src in sources:
        bases.append(bases[-1] + src.shape[0])
    q0, uk0, kv0, uv0, g0, u0, d0, o0, expand0 = bases
    lhs0 = expand0 + n_expand * _LANES // _SLAB

    groups = [
        (src, base, _pages(src.shape[0], _CACHE_SPACING if src is ckv_hbm else _SPACING))
        for src, base in zip(sources, bases)
    ]
    first_wo = len(groups) - 1
    wo_pages = groups.pop()[2]
    last = [
        (start, size) for start, size in wo_pages
        if size == _PAGE and start % (M // _SLAB) % _PAGE == 0
        and start % (M // _SLAB) + size <= M // _SLAB
    ][-_LOW_AT_END:]
    wo_pages = [page for page in wo_pages if page not in last] + last
    cuts = [len(wo_pages) - sum(_WO_GROUPS[i:]) for i in range(len(_WO_GROUPS) + 1)]
    groups += [(wo_hbm, o0, wo_pages[a:b]) for a, b in zip([0] + cuts[:-1], cuts)]
    stream = _Stream(groups, buf, sems)

    def flat(start, n):
        return buf[start:start + n].reshape(n * _SLAB, _LANES)

    def head_group(base, row0, n, g):
        return buf[base + row0:base + row0 + n, g * _HG:(g + 1) * _HG, :].reshape(n * _HG, D)

    def column_tile(base, width, row0, n, j):
        per_band = width // _LANES * _TILE_ROWS // _SLAB
        slab, row = divmod(j * _TILE_ROWS, _SLAB)
        first = base + row0 // _TILE_ROWS * per_band + slab
        bands = pl.ds(first, n // _TILE_ROWS, stride=per_band)
        return buf[bands, row:row + _TILE_ROWS, :].reshape(n, _LANES)

    def expand(t):
        return flat(expand0 + t * _LANES // _SLAB, _LANES // _SLAB)

    x_cp = pltpu.make_async_copy(x_hbm, x_v, small_sems.at[0])
    wr_cp = pltpu.make_async_copy(wr_hbm, wr_v, small_sems.at[1])
    stream.advance(_LEAD // 2)
    x_cp.start()
    wr_cp.start()
    stream.advance(_QUEUE)

    square = (_LANES, _LANES)
    for t in range(n_expand):
        e = _iota(square, 1) // _HG + t * per_tile == _iota(square, 0)
        first = expand0 + t * _LANES // _SLAB
        buf[first:first + _LANES // _SLAB] = e.astype(_BF16).reshape(-1, _SLAB, _LANES)
        if t % 4 == 3:
            stream.advance()
    own_head = _iota((rows, _LANES), 1) % _HG == _iota((rows, _LANES), 0) % _HG

    x_cp.wait()
    wr_cp.wait()
    x = _pad_rows(x_v[...].astype(_F32))
    xc = x - jnp.mean(x, axis=-1, keepdims=True)
    xn_lo = (xc / jnp.sqrt(jnp.mean(xc * xc, axis=-1, keepdims=True) + 1e-5)).astype(_BF16)
    xn = xn_lo.astype(_F32)
    wr = wr_v[...].astype(_F32).reshape(1, M)
    route = jax.nn.sigmoid(jnp.sum(xn * wr, axis=-1, keepdims=True))

    lhs_slabs = rows // _SLAB
    for t in range(M // per_tile):
        m0 = t // n_expand * _LANES
        n = min(_LANES, M - m0)
        rep = _dot(xn_lo[:, m0:m0 + n], expand(t % n_expand)[:n])
        rep = jnp.concatenate(
            [jnp.broadcast_to(rep[b:b + 1], (_HG, _LANES)) for b in range(B)], axis=0
        )
        first = lhs0 + t * lhs_slabs
        buf[first:first + lhs_slabs] = (
            jnp.where(own_head, rep, 0.0).astype(_BF16).reshape(lhs_slabs, _SLAB, _LANES)
        )
        if t % 8 == 7:
            stream.advance()
    stream.wait(0)
    q = [jnp.zeros((rows, D), _F32) for _ in range(n_groups)]
    for t in range(M // per_tile):
        lhs = flat(lhs0 + t * lhs_slabs, lhs_slabs)
        for g in range(n_groups):
            q[g] = q[g] + _dot(lhs, head_group(q0, t * per_tile, per_tile, g))
        if t % 6 == 5:
            stream.advance()

    stream.wait(1)
    q_lat = []
    for g in range(n_groups):
        qg = q[g].astype(_BF16)
        tiles = []
        for c0 in range(0, Dc, _LANES):
            acc = jnp.zeros((rows, _LANES), _F32)
            for t in range(n_expand):
                full = _dot_nt(qg, head_group(uk0, c0 + t * per_tile, per_tile, g))
                acc = acc + _dot_nt(jnp.where(own_head, full, 0.0).astype(_BF16), expand(t))
                if t % 8 == 7:
                    stream.advance()
            tiles.append(acc.astype(_BF16))
        q_lat.append(tiles)

    qk_keys, pv_keys = 512, 1024
    lat_tiles = range(Dc // _LANES)

    def scores(b):
        qb = [
            jnp.concatenate([q_lat[g][j][b * _HG:(b + 1) * _HG] for g in range(n_groups)], axis=0)
            for j in lat_tiles
        ]
        chunks = []
        for k0 in range(b * keys, (b + 1) * keys, qk_keys):
            parts = [_dot_nt(qb[j], column_tile(kv0, Dc, k0, qk_keys, j)) for j in lat_tiles]
            chunks.append(sum(parts[1:], parts[0]))
            stream.advance()
        return jnp.concatenate(chunks, axis=1) * (D ** -0.5)

    def attend(b, s):
        p = jnp.exp(s - jnp.max(s, axis=-1, keepdims=True))
        denom = jnp.sum(p, axis=-1, keepdims=True)
        p = p.astype(_BF16)
        acc = [jnp.zeros((heads, _LANES), _F32) for _ in lat_tiles]
        for k0 in range(0, keys, pv_keys):
            acc = [
                a + _dot(p[:, k0:k0 + pv_keys], column_tile(kv0, Dc, b * keys + k0, pv_keys, j))
                for j, a in enumerate(acc)
            ]
            stream.advance()
        return [(a / denom).astype(_BF16) for a in acc]

    stream.wait(2)
    lat = []
    s = scores(0)
    for b in range(B):
        ahead = scores(b + 1) if b + 1 < B else None
        lat.append(attend(b, s))
        s = ahead

    stream.wait(3)
    for g in range(n_groups):
        ctx = jnp.zeros((rows, D), _F32)
        for j in range(Dc // _LANES):
            lg = jnp.concatenate([lb[j][g * _HG:(g + 1) * _HG] for lb in lat], axis=0)
            for t in range(n_expand):
                lhs = jnp.where(own_head, _dot(lg, expand(t)), 0.0).astype(_BF16)
                ctx = ctx + _dot(lhs, head_group(uv0, j * _LANES + t * per_tile, per_tile, g))
                if t % 8 == 7:
                    stream.advance()
        ctx_v[g * rows:(g + 1) * rows, :] = ctx

    def project(base):
        tiles = []
        for j in range(hidden_dim // _LANES):
            tiles.append(_dot(xn_lo, column_tile(base, hidden_dim, 0, M, j)))
            if j % 6 == 5:
                stream.advance()
        return tiles

    stream.wait(4)
    gate = [jax.nn.silu(v) for v in project(g0)]
    stream.wait(5)
    hidden = [(a * v).astype(_BF16) for a, v in zip(gate, project(u0))]
    stream.wait(6)
    y = jnp.zeros(x.shape, _F32)
    for j, hj in enumerate(hidden):
        y = y + _dot_nt(hj, column_tile(d0, hidden_dim, 0, M, j))
        if j % 3 == 2:
            stream.advance()
    mixed = jax.nn.silu(xn + (xn * 0.0 + y * route))

    def ctx_rows(h):
        first = h // _HG * rows + h % _HG
        return _pad_rows(ctx_v[pl.ds(first, B, stride=_HG), :]).astype(_BF16)

    def per_head(pages):
        for start, size in pages:
            while size:
                h, m_slab = divmod(start, M // _SLAB)
                n = min(size, M // _SLAB - m_slab)
                yield h, m_slab * _SLAB, start, n
                start, size = start + n, size - n

    def place(v, m0):
        pads = [jnp.zeros((v.shape[0], w), v.dtype) for w in (m0, M - m0 - v.shape[1])]
        return jnp.concatenate([a for a in (pads[0], v, pads[1]) if a.shape[1]], axis=1)

    lane_tiles = [(m0, min(_LANES, M - m0)) for m0 in range(0, M, _LANES)]
    s = {tile: jnp.zeros((x.shape[0], tile[1]), _F32) for tile in lane_tiles}
    shifted = {}
    for g in range(first_wo, len(groups)):
        work = list(per_head(groups[g][2]))
        lhs = {h: ctx_rows(h) for h in sorted({h for h, _, _, _ in work})}
        stream.wait(g)
        for (m0, _), v in shifted.items():
            wide = place(v, m0)
            s = {(a, w): acc + wide[:, a:a + w] for (a, w), acc in s.items()}
        shifted = {}
        for h, m0, start, n in work:
            tile = (m0, n * _SLAB)
            into = s if tile in s else shifted
            part = _dot_nt(lhs[h], flat(o0 + start, n))
            into[tile] = into[tile] + part if tile in into else part
    assert not shifted

    out = x + jnp.concatenate([s[tile] for tile in lane_tiles], axis=1) * mixed
    out_v[...] = out.astype(out_v.dtype)[:B]
    out_cp = pltpu.make_async_copy(out_v, out_hbm, small_sems.at[0])
    out_cp.start()
    out_cp.wait()


def _slabs(w):
    r, c = w.shape
    w = w.reshape(r // _TILE_ROWS, _TILE_ROWS, c // _LANES, _LANES)
    return w.transpose(0, 2, 1, 3).reshape(-1, _SLAB, _LANES)


@jax.jit
def pallas_recurrent_scan__compressed_kv_cla__moe_arch_mod__decode_kernel(
    A_x: jax.Array,
    A_c_kv: jax.Array,
    A_w_q: jax.Array,
    A_w_uk: jax.Array,
    A_w_uv: jax.Array,
    A_w_o: jax.Array,
    B_x: jax.Array,
    B_w_r: jax.Array,
    B_w_gate: jax.Array,
    B_w_up: jax.Array,
    B_w_down: jax.Array,
):
    del B_x
    B, Sq, M = A_x.shape
    _, Sk, Dc = A_c_kv.shape
    _, H, D = A_w_q.shape
    assert Sq == 1 and H == _SLAB and D == _LANES

    x = A_x.reshape(B, M)
    streamed = [
        A_w_q,
        A_w_uk,
        _slabs(A_c_kv.reshape(B * Sk, Dc)),
        A_w_uv,
        _slabs(B_w_gate),
        _slabs(B_w_up),
        _slabs(B_w_down.T),
        jnp.transpose(A_w_o, (0, 2, 1)).reshape(-1, _SLAB, _LANES),
    ]
    n_slabs = sum(w.shape[0] for w in streamed) + (_HG * _LANES + M * B * _HG * _HG // D) // _SLAB

    def kernel(*refs):
        _kernel(*refs, heads=H, keys=Sk, hidden_dim=B_w_gate.shape[1])

    hbm = pl.BlockSpec(memory_space=pltpu.HBM)
    out = pl.pallas_call(
        kernel,
        out_shape=jax.ShapeDtypeStruct((B, M), A_x.dtype),
        in_specs=[hbm] * (2 + len(streamed)),
        out_specs=hbm,
        scratch_shapes=[
            pltpu.VMEM((n_slabs, _SLAB, _LANES), _BF16),
            pltpu.VMEM(x.shape, x.dtype),
            pltpu.VMEM(B_w_r.shape, B_w_r.dtype),
            pltpu.VMEM(x.shape, x.dtype),
            pltpu.VMEM((B * H, D), _F32),
            pltpu.SemaphoreType.DMA((len(streamed) + len(_WO_GROUPS),)),
            pltpu.SemaphoreType.DMA((2,)),
        ],
        compiler_params=pltpu.CompilerParams(
            vmem_limit_bytes=96 * 1024 * 1024, disable_semaphore_checks=True
        ),
    )(x, B_w_r, *streamed)
    return out.reshape(B, Sq, M)
```

```python
import jax
import jax.numpy as jnp
from jax import lax
import jax.experimental.pallas as pl
import jax.experimental.pallas.tpu as pltpu

_F32 = jnp.float32
_BF16 = jnp.bfloat16
_LANES = 128
_TILE_ROWS = 8
_SLAB = 32
_HG = 16

_WQ, _WUK, _CKV, _WUV, _WG, _WU, _WD, _WO = range(8)

_PAGE = 4
_PAGE_START = 2
_SPACING = (16, 16, 32, 16, 16, 16, 16, 16)
_WO_GROUPS = (36, 12, 8, 4, 4, 4)
_LOW_PER_HIGH = 3
_LEAD = 26
_LOW_AT_END = 20
_STEP = 5
_QUEUE = 82


def _dot(a, b):
    return jnp.dot(a, b, preferred_element_type=_F32)


def _dot_nt(a, b):
    return lax.dot_general(a, b, (((1,), (1,)), ((), ())), preferred_element_type=_F32)


def _iota(shape, axis):
    return lax.broadcasted_iota(jnp.int32, shape, axis)


def _pad_rows(v):
    return jnp.concatenate([v, jnp.zeros((8 - v.shape[0], v.shape[1]), v.dtype)], axis=0)


def _pages(n_slabs, spacing):
    whole = list(range(_PAGE_START, n_slabs - _PAGE + 1, _PAGE))
    ragged = [(whole[-1] + _PAGE, n_slabs), (0, _PAGE_START)]
    return [(a, b - a) for a, b in ragged if b > a] + [
        (start, _PAGE) for i in range(spacing) for start in whole[i::spacing]
    ]


class _Stream:
    def __init__(self, order, groups, buf, sems):
        self.order, self.groups, self.buf, self.sems = order, groups, buf, sems
        is_high = [
            i % (_LOW_PER_HIGH + 1) == 0 and i < len(order) - _LOW_AT_END
            for i in range(len(order))
        ]
        high = [c + (0,) for c, h in zip(order, is_high) if h]
        low = [c + (1,) for c, h in zip(order, is_high) if not h]
        self.todo, low = low[:_LEAD], low[_LEAD:]
        for i, c in enumerate(high):
            self.todo += [c] + low[i * _LOW_PER_HIGH:(i + 1) * _LOW_PER_HIGH]
        self.todo += low[len(high) * _LOW_PER_HIGH:]
        self.ready = {}
        for i, (g, _, _, priority) in enumerate(self.todo):
            self.ready[g] = max(self.ready.get(g, 0), i + (_QUEUE if priority else 8))
        self.done = 0

    def _copy(self, g, start, size):
        src, base = self.groups[g]
        return pltpu.make_async_copy(
            src.at[pl.ds(start, size)], self.buf.at[pl.ds(base + start, size)], self.sems.at[g]
        )

    def advance(self, count=None):
        count = _STEP if count is None else count
        for *copy, priority in self.todo[self.done:self.done + count]:
            self._copy(*copy).start(priority=priority)
        self.done = min(self.done + count, len(self.todo))

    def wait(self, g):
        self.advance(max(self.ready[g] - self.done, 0))
        src, base = self.groups[g]
        copies = [c for c in self.order if c[0] == g]
        if sum(size for _, _, size in copies) == src.shape[0]:
            filled = self.buf.at[pl.ds(base, src.shape[0])]
            pltpu.make_async_copy(filled, filled, self.sems.at[g]).wait()
        else:
            for copy in copies:
                self._copy(*copy).wait()


def _kernel(
    x_hbm, wr_hbm, wq_hbm, wuk_hbm, ckv_hbm, wuv_hbm, wg_hbm, wu_hbm, wd_hbm, wo_hbm,
    out_hbm,
    buf, x_v, wr_v, out_v, ctx_v, sems, small_sems,
    *, heads, keys, hidden_dim,
):
    B, M = x_v.shape
    D = _LANES
    Dc = wuk_hbm.shape[0]
    n_groups = heads // _HG
    rows = B * _HG
    per_tile = _LANES // _HG
    n_expand = _LANES // per_tile

    sources = [wq_hbm, wuk_hbm, ckv_hbm, wuv_hbm, wg_hbm, wu_hbm, wd_hbm, wo_hbm]
    bases = [0]
    for src in sources:
        bases.append(bases[-1] + src.shape[0])
    q0, uk0, kv0, uv0, g0, u0, d0, o0, expand0 = bases
    lhs0 = expand0 + n_expand * _LANES // _SLAB

    groups = list(zip(sources, bases))
    order = [(g, *page) for g in range(_WO) for page in _pages(sources[g].shape[0], _SPACING[g])]
    head_slabs = M // _SLAB
    wo_pages = _pages(wo_hbm.shape[0], _SPACING[_WO])
    last = [
        (start, size) for start, size in wo_pages
        if size == _PAGE and start % head_slabs % _PAGE == 0
        and start % head_slabs + size <= head_slabs
    ][-_LOW_AT_END:]
    wo_pages = [page for page in wo_pages if page not in last] + last
    cuts = [len(wo_pages) - sum(_WO_GROUPS[i:]) for i in range(len(_WO_GROUPS) + 1)]
    wo_groups = [wo_pages[a:b] for a, b in zip([0] + cuts[:-1], cuts)]
    groups += [groups[_WO]] * len(_WO_GROUPS)
    order += [(g, *page) for g, pages in enumerate(wo_groups, _WO) for page in pages]
    stream = _Stream(order, groups, buf, sems)

    def flat(start, n):
        return buf[start:start + n].reshape(n * _SLAB, _LANES)

    def head_group(base, row0, n, g):
        return buf[base + row0:base + row0 + n, g * _HG:(g + 1) * _HG, :].reshape(n * _HG, D)

    def column_tile(base, width, row0, n, j):
        per_band = width // _LANES * _TILE_ROWS // _SLAB
        slab, row = divmod(j * _TILE_ROWS, _SLAB)
        first = base + row0 // _TILE_ROWS * per_band + slab
        bands = pl.ds(first, n // _TILE_ROWS, stride=per_band)
        return buf[bands, row:row + _TILE_ROWS, :].reshape(n, _LANES)

    def expand(t):
        return flat(expand0 + t * _LANES // _SLAB, _LANES // _SLAB)

    x_cp = pltpu.make_async_copy(x_hbm, x_v, small_sems.at[0])
    wr_cp = pltpu.make_async_copy(wr_hbm, wr_v, small_sems.at[1])
    stream.advance(_LEAD // 2)
    x_cp.start()
    wr_cp.start()
    stream.advance(_QUEUE)

    square = (_LANES, _LANES)
    for t in range(n_expand):
        e = _iota(square, 1) // _HG + t * per_tile == _iota(square, 0)
        first = expand0 + t * _LANES // _SLAB
        buf[first:first + _LANES // _SLAB] = e.astype(_BF16).reshape(-1, _SLAB, _LANES)
        if t % 4 == 3:
            stream.advance()
    own_head = _iota((rows, _LANES), 1) % _HG == _iota((rows, _LANES), 0) % _HG

    x_cp.wait()
    wr_cp.wait()
    x = _pad_rows(x_v[...].astype(_F32))
    xc = x - jnp.mean(x, axis=-1, keepdims=True)
    xn_lo = (xc / jnp.sqrt(jnp.mean(xc * xc, axis=-1, keepdims=True) + 1e-5)).astype(_BF16)
    xn = xn_lo.astype(_F32)
    wr = wr_v[...].astype(_F32).reshape(1, M)
    route = jax.nn.sigmoid(jnp.sum(xn * wr, axis=-1, keepdims=True))

    lhs_slabs = rows // _SLAB
    for t in range(M // per_tile):
        m0 = t // n_expand * _LANES
        n = min(_LANES, M - m0)
        rep = _dot(xn_lo[:, m0:m0 + n], expand(t % n_expand)[:n])
        rep = jnp.concatenate(
            [jnp.broadcast_to(rep[b:b + 1], (_HG, _LANES)) for b in range(B)], axis=0
        )
        first = lhs0 + t * lhs_slabs
        buf[first:first + lhs_slabs] = (
            jnp.where(own_head, rep, 0.0).astype(_BF16).reshape(lhs_slabs, _SLAB, _LANES)
        )
        if t % 8 == 7:
            stream.advance()
    stream.wait(_WQ)
    q = [jnp.zeros((rows, D), _F32) for _ in range(n_groups)]
    for t in range(M // per_tile):
        lhs = flat(lhs0 + t * lhs_slabs, lhs_slabs)
        for g in range(n_groups):
            q[g] = q[g] + _dot(lhs, head_group(q0, t * per_tile, per_tile, g))
        if t % 6 == 5:
            stream.advance()

    stream.wait(_WUK)
    q_lat = []
    for g in range(n_groups):
        qg = q[g].astype(_BF16)
        tiles = []
        for c0 in range(0, Dc, _LANES):
            acc = jnp.zeros((rows, _LANES), _F32)
            for t in range(n_expand):
                full = _dot_nt(qg, head_group(uk0, c0 + t * per_tile, per_tile, g))
                acc = acc + _dot_nt(jnp.where(own_head, full, 0.0).astype(_BF16), expand(t))
                if t % 8 == 7:
                    stream.advance()
            tiles.append(acc.astype(_BF16))
        q_lat.append(tiles)

    qk_keys, pv_keys = 512, 1024
    lat_tiles = range(Dc // _LANES)

    def scores(b):
        qb = [
            jnp.concatenate([q_lat[g][j][b * _HG:(b + 1) * _HG] for g in range(n_groups)], axis=0)
            for j in lat_tiles
        ]
        chunks = []
        for k0 in range(b * keys, (b + 1) * keys, qk_keys):
            parts = [_dot_nt(qb[j], column_tile(kv0, Dc, k0, qk_keys, j)) for j in lat_tiles]
            chunks.append(sum(parts[1:], parts[0]))
            stream.advance()
        return jnp.concatenate(chunks, axis=1) * (D ** -0.5)

    def attend(b, s):
        p = jnp.exp(s - jnp.max(s, axis=-1, keepdims=True))
        denom = jnp.sum(p, axis=-1, keepdims=True)
        p = p.astype(_BF16)
        acc = [jnp.zeros((heads, _LANES), _F32) for _ in lat_tiles]
        for k0 in range(0, keys, pv_keys):
            acc = [
                a + _dot(p[:, k0:k0 + pv_keys], column_tile(kv0, Dc, b * keys + k0, pv_keys, j))
                for j, a in enumerate(acc)
            ]
            stream.advance()
        return [(a / denom).astype(_BF16) for a in acc]

    stream.wait(_CKV)
    lat = []
    s = scores(0)
    for b in range(B):
        ahead = scores(b + 1) if b + 1 < B else None
        lat.append(attend(b, s))
        s = ahead

    stream.wait(_WUV)
    for g in range(n_groups):
        ctx = jnp.zeros((rows, D), _F32)
        for j in range(Dc // _LANES):
            lg = jnp.concatenate([lb[j][g * _HG:(g + 1) * _HG] for lb in lat], axis=0)
            for t in range(n_expand):
                lhs = jnp.where(own_head, _dot(lg, expand(t)), 0.0).astype(_BF16)
                ctx = ctx + _dot(lhs, head_group(uv0, j * _LANES + t * per_tile, per_tile, g))
                if t % 8 == 7:
                    stream.advance()
        ctx_v[g * rows:(g + 1) * rows, :] = ctx

    def project(base):
        tiles = []
        for j in range(hidden_dim // _LANES):
            tiles.append(_dot(xn_lo, column_tile(base, hidden_dim, 0, M, j)))
            if j % 6 == 5:
                stream.advance()
        return tiles

    stream.wait(_WG)
    gate = [jax.nn.silu(v) for v in project(g0)]
    stream.wait(_WU)
    hidden = [(a * v).astype(_BF16) for a, v in zip(gate, project(u0))]
    stream.wait(_WD)
    y = jnp.zeros(x.shape, _F32)
    for j, hj in enumerate(hidden):
        y = y + _dot_nt(hj, column_tile(d0, hidden_dim, 0, M, j))
        if j % 3 == 2:
            stream.advance()
    mixed = jax.nn.silu(xn + (xn * 0.0 + y * route))

    def ctx_rows(h):
        first = h // _HG * rows + h % _HG
        return _pad_rows(ctx_v[pl.ds(first, B, stride=_HG), :]).astype(_BF16)

    def per_head(pages):
        for start, size in pages:
            while size:
                h, m_slab = divmod(start, head_slabs)
                n = min(size, head_slabs - m_slab)
                yield h, m_slab * _SLAB, start, n
                start, size = start + n, size - n

    def place(v, m0):
        pads = [jnp.zeros((v.shape[0], w), v.dtype) for w in (m0, M - m0 - v.shape[1])]
        return jnp.concatenate([a for a in (pads[0], v, pads[1]) if a.shape[1]], axis=1)

    lane_tiles = [(m0, min(_LANES, M - m0)) for m0 in range(0, M, _LANES)]
    s = {tile: jnp.zeros((x.shape[0], tile[1]), _F32) for tile in lane_tiles}
    shifted = {}
    for g, pages in enumerate(wo_groups, _WO):
        work = list(per_head(pages))
        lhs = {h: ctx_rows(h) for h in sorted({h for h, _, _, _ in work})}
        stream.wait(g)
        for (m0, _), v in shifted.items():
            wide = place(v, m0)
            s = {(a, w): acc + wide[:, a:a + w] for (a, w), acc in s.items()}
        shifted = {}
        for h, m0, start, n in work:
            tile = (m0, n * _SLAB)
            into = s if tile in s else shifted
            part = _dot_nt(lhs[h], flat(o0 + start, n))
            into[tile] = into[tile] + part if tile in into else part
    assert not shifted

    out = x + jnp.concatenate([s[tile] for tile in lane_tiles], axis=1) * mixed
    out_v[...] = out.astype(out_v.dtype)[:B]
    out_cp = pltpu.make_async_copy(out_v, out_hbm, small_sems.at[0])
    out_cp.start()
    out_cp.wait()


def _slabs(w):
    r, c = w.shape
    w = w.reshape(r // _TILE_ROWS, _TILE_ROWS, c // _LANES, _LANES)
    return w.transpose(0, 2, 1, 3).reshape(-1, _SLAB, _LANES)


@jax.jit
def pallas_recurrent_scan__compressed_kv_cla__moe_arch_mod__decode_kernel(
    A_x: jax.Array,
    A_c_kv: jax.Array,
    A_w_q: jax.Array,
    A_w_uk: jax.Array,
    A_w_uv: jax.Array,
    A_w_o: jax.Array,
    B_x: jax.Array,
    B_w_r: jax.Array,
    B_w_gate: jax.Array,
    B_w_up: jax.Array,
    B_w_down: jax.Array,
):
    del B_x
    B, Sq, M = A_x.shape
    _, Sk, Dc = A_c_kv.shape
    _, H, D = A_w_q.shape
    assert Sq == 1 and H == _SLAB and D == _LANES

    x = A_x.reshape(B, M)
    streamed = [
        A_w_q,
        A_w_uk,
        _slabs(A_c_kv.reshape(B * Sk, Dc)),
        A_w_uv,
        _slabs(B_w_gate),
        _slabs(B_w_up),
        _slabs(B_w_down.T),
        jnp.transpose(A_w_o, (0, 2, 1)).reshape(-1, _SLAB, _LANES),
    ]
    n_slabs = sum(w.shape[0] for w in streamed) + (_HG * _LANES + M * B * _HG * _HG // D) // _SLAB

    def kernel(*refs):
        _kernel(*refs, heads=H, keys=Sk, hidden_dim=B_w_gate.shape[1])

    hbm = pl.BlockSpec(memory_space=pltpu.HBM)
    out = pl.pallas_call(
        kernel,
        out_shape=jax.ShapeDtypeStruct((B, M), A_x.dtype),
        in_specs=[hbm] * (2 + len(streamed)),
        out_specs=hbm,
        scratch_shapes=[
            pltpu.VMEM((n_slabs, _SLAB, _LANES), _BF16),
            pltpu.VMEM(x.shape, x.dtype),
            pltpu.VMEM(B_w_r.shape, B_w_r.dtype),
            pltpu.VMEM(x.shape, x.dtype),
            pltpu.VMEM((B * H, D), _F32),
            pltpu.SemaphoreType.DMA((len(streamed) + len(_WO_GROUPS),)),
            pltpu.SemaphoreType.DMA((2,)),
        ],
        compiler_params=pltpu.CompilerParams(
            vmem_limit_bytes=96 * 1024 * 1024, disable_semaphore_checks=True
        ),
    )(x, B_w_r, *streamed)
    return out.reshape(B, Sq, M)
```

```python
import jax
import jax.numpy as jnp
from jax import lax
import jax.experimental.pallas as pl
import jax.experimental.pallas.tpu as pltpu

_F32 = jnp.float32
_BF16 = jnp.bfloat16
_LANES = 128
_TILE_ROWS = 8
_SLAB = 32
_HG = 16

_WQ, _WUK, _CKV, _WUV, _WG, _WU, _WD, _WO = range(8)

_PAGE = 4
_PAGE_START = 2
_SPACING = (16, 16, 32, 16, 16, 16, 16, 16)
_WO_GROUPS = (36, 12, 8, 4, 4, 4)
_LOW_PER_HIGH = 3
_LEAD = 26
_LOW_AT_END = 20
_STEP = 5
_QUEUE = 82


def _dot(a, b):
    return jnp.dot(a, b, preferred_element_type=_F32)


def _dot_nt(a, b):
    return lax.dot_general(a, b, (((1,), (1,)), ((), ())), preferred_element_type=_F32)


def _iota(shape, axis):
    return lax.broadcasted_iota(jnp.int32, shape, axis)


def _pad_rows(v):
    return jnp.concatenate([v, jnp.zeros((8 - v.shape[0], v.shape[1]), v.dtype)], axis=0)


def _pages(n_slabs, spacing):
    whole = list(range(_PAGE_START, n_slabs - _PAGE + 1, _PAGE))
    ragged = [(whole[-1] + _PAGE, n_slabs), (0, _PAGE_START)]
    return [(a, b - a) for a, b in ragged if b > a] + [
        (start, _PAGE) for i in range(spacing) for start in whole[i::spacing]
    ]


class _Stream:
    def __init__(self, order, groups, buf, sems):
        self.order, self.groups, self.buf, self.sems = order, groups, buf, sems
        is_high = [
            i % (_LOW_PER_HIGH + 1) == 0 and i < len(order) - _LOW_AT_END
            for i in range(len(order))
        ]
        high = [c + (0,) for c, h in zip(order, is_high) if h]
        low = [c + (1,) for c, h in zip(order, is_high) if not h]
        self.todo, low = low[:_LEAD], low[_LEAD:]
        for i, c in enumerate(high):
            self.todo += [c] + low[i * _LOW_PER_HIGH:(i + 1) * _LOW_PER_HIGH]
        self.todo += low[len(high) * _LOW_PER_HIGH:]
        self.ready = {}
        for i, (g, _, _, priority) in enumerate(self.todo):
            self.ready[g] = max(self.ready.get(g, 0), i + (_QUEUE if priority else 8))
        self.done = 0

    def _copy(self, g, start, size):
        src, base = self.groups[g]
        return pltpu.make_async_copy(
            src.at[pl.ds(start, size)], self.buf.at[pl.ds(base + start, size)], self.sems.at[g]
        )

    def advance(self, count=None):
        count = _STEP if count is None else count
        for *copy, priority in self.todo[self.done:self.done + count]:
            self._copy(*copy).start(priority=priority)
        self.done = min(self.done + count, len(self.todo))

    def wait(self, g):
        self.advance(max(self.ready[g] - self.done, 0))
        src, base = self.groups[g]
        copies = [c for c in self.order if c[0] == g]
        if sum(size for _, _, size in copies) == src.shape[0]:
            filled = self.buf.at[pl.ds(base, src.shape[0])]
            pltpu.make_async_copy(filled, filled, self.sems.at[g]).wait()
        else:
            for copy in copies:
                self._copy(*copy).wait()


def _kernel(
    x_hbm, wr_hbm, wq_hbm, wuk_hbm, ckv_hbm, wuv_hbm, wg_hbm, wu_hbm, wd_hbm, wo_hbm,
    out_hbm,
    buf, x_v, wr_v, out_v, ctx_v, sems, small_sems,
    *, heads, keys, hidden_dim,
):
    B, M = x_v.shape
    D = _LANES
    Dc = wuk_hbm.shape[0]
    n_groups = heads // _HG
    rows = B * _HG
    per_tile = _LANES // _HG
    n_expand = _LANES // per_tile

    sources = [wq_hbm, wuk_hbm, ckv_hbm, wuv_hbm, wg_hbm, wu_hbm, wd_hbm, wo_hbm]
    bases = [0]
    for src in sources:
        bases.append(bases[-1] + src.shape[0])
    q0, uk0, kv0, uv0, g0, u0, d0, o0, expand0 = bases
    lhs0 = expand0 + n_expand * _LANES // _SLAB

    groups = list(zip(sources, bases))
    order = [(g, *page) for g in range(_WO) for page in _pages(sources[g].shape[0], _SPACING[g])]
    head_slabs = M // _SLAB
    wo_pages = _pages(wo_hbm.shape[0], _SPACING[_WO])
    last = [
        (start, size) for start, size in wo_pages
        if size == _PAGE and start % head_slabs % _PAGE == 0
        and start % head_slabs + size <= head_slabs
    ][-_LOW_AT_END:]
    wo_pages = [page for page in wo_pages if page not in last] + last
    cuts = [len(wo_pages) - sum(_WO_GROUPS[i:]) for i in range(len(_WO_GROUPS) + 1)]
    wo_groups = [wo_pages[a:b] for a, b in zip([0] + cuts[:-1], cuts)]
    groups += [groups[_WO]] * len(_WO_GROUPS)
    order += [(g, *page) for g, pages in enumerate(wo_groups, _WO) for page in pages]
    stream = _Stream(order, groups, buf, sems)

    def flat(start, n):
        return buf[start:start + n].reshape(n * _SLAB, _LANES)

    def head_group(base, row0, n, g):
        return buf[base + row0:base + row0 + n, g * _HG:(g + 1) * _HG, :].reshape(n * _HG, D)

    def column_tile(base, width, row0, n, j):
        per_band = width // _LANES * _TILE_ROWS // _SLAB
        slab, row = divmod(j * _TILE_ROWS, _SLAB)
        first = base + row0 // _TILE_ROWS * per_band + slab
        rows8 = slice(row, row + _TILE_ROWS)
        if per_band == 1:
            return buf[first:first + n // _TILE_ROWS, rows8, :].reshape(n, _LANES)
        return jnp.concatenate(
            [buf[first + i * per_band, rows8, :] for i in range(n // _TILE_ROWS)], axis=0
        )

    def expand(t):
        return flat(expand0 + t * _LANES // _SLAB, _LANES // _SLAB)

    x_cp = pltpu.make_async_copy(x_hbm, x_v, small_sems.at[0])
    wr_cp = pltpu.make_async_copy(wr_hbm, wr_v, small_sems.at[1])
    stream.advance(_LEAD // 2)
    x_cp.start()
    wr_cp.start()
    stream.advance(_QUEUE)

    square = (_LANES, _LANES)
    for t in range(n_expand):
        e = _iota(square, 1) // _HG + t * per_tile == _iota(square, 0)
        first = expand0 + t * _LANES // _SLAB
        buf[first:first + _LANES // _SLAB] = e.astype(_BF16).reshape(-1, _SLAB, _LANES)
        if t % 4 == 3:
            stream.advance()
    own_head = _iota((rows, _LANES), 1) % _HG == _iota((rows, _LANES), 0) % _HG

    x_cp.wait()
    wr_cp.wait()
    x = _pad_rows(x_v[...].astype(_F32))
    xc = x - jnp.mean(x, axis=-1, keepdims=True)
    xn_lo = (xc / jnp.sqrt(jnp.mean(xc * xc, axis=-1, keepdims=True) + 1e-5)).astype(_BF16)
    xn = xn_lo.astype(_F32)
    wr = wr_v[...].astype(_F32).reshape(1, M)
    route = jax.nn.sigmoid(jnp.sum(xn * wr, axis=-1, keepdims=True))

    lhs_slabs = rows // _SLAB
    for t in range(M // per_tile):
        m0 = t // n_expand * _LANES
        n = min(_LANES, M - m0)
        rep = _dot(xn_lo[:, m0:m0 + n], expand(t % n_expand)[:n])
        rep = jnp.concatenate(
            [jnp.broadcast_to(rep[b:b + 1], (_HG, _LANES)) for b in range(B)], axis=0
        )
        first = lhs0 + t * lhs_slabs
        buf[first:first + lhs_slabs] = (
            jnp.where(own_head, rep, 0.0).astype(_BF16).reshape(lhs_slabs, _SLAB, _LANES)
        )
        if t % 8 == 7:
            stream.advance()
    stream.wait(_WQ)
    q = [jnp.zeros((rows, D), _F32) for _ in range(n_groups)]
    for t in range(M // per_tile):
        lhs = flat(lhs0 + t * lhs_slabs, lhs_slabs)
        for g in range(n_groups):
            q[g] = q[g] + _dot(lhs, head_group(q0, t * per_tile, per_tile, g))
        if t % 6 == 5:
            stream.advance()

    stream.wait(_WUK)
    q_lat = []
    for g in range(n_groups):
        qg = q[g].astype(_BF16)
        tiles = []
        for c0 in range(0, Dc, _LANES):
            acc = jnp.zeros((rows, _LANES), _F32)
            for t in range(n_expand):
                full = _dot_nt(qg, head_group(uk0, c0 + t * per_tile, per_tile, g))
                acc = acc + _dot_nt(jnp.where(own_head, full, 0.0).astype(_BF16), expand(t))
                if t % 8 == 7:
                    stream.advance()
            tiles.append(acc.astype(_BF16))
        q_lat.append(tiles)

    qk_keys, pv_keys = 512, 1024
    lat_tiles = range(Dc // _LANES)

    def scores(b):
        qb = [
            jnp.concatenate([q_lat[g][j][b * _HG:(b + 1) * _HG] for g in range(n_groups)], axis=0)
            for j in lat_tiles
        ]
        chunks = []
        for k0 in range(b * keys, (b + 1) * keys, qk_keys):
            parts = [_dot_nt(qb[j], column_tile(kv0, Dc, k0, qk_keys, j)) for j in lat_tiles]
            chunks.append(sum(parts[1:], parts[0]))
            stream.advance()
        return jnp.concatenate(chunks, axis=1) * (D ** -0.5)

    def attend(b, s):
        p = jnp.exp(s - jnp.max(s, axis=-1, keepdims=True))
        denom = jnp.sum(p, axis=-1, keepdims=True)
        p = p.astype(_BF16)
        acc = [jnp.zeros((heads, _LANES), _F32) for _ in lat_tiles]
        for k0 in range(0, keys, pv_keys):
            acc = [
                a + _dot(p[:, k0:k0 + pv_keys], column_tile(kv0, Dc, b * keys + k0, pv_keys, j))
                for j, a in enumerate(acc)
            ]
            stream.advance()
        return [(a / denom).astype(_BF16) for a in acc]

    stream.wait(_CKV)
    lat = []
    s = scores(0)
    for b in range(B):
        ahead = scores(b + 1) if b + 1 < B else None
        lat.append(attend(b, s))
        s = ahead

    stream.wait(_WUV)
    for g in range(n_groups):
        ctx = jnp.zeros((rows, D), _F32)
        for j in range(Dc // _LANES):
            lg = jnp.concatenate([lb[j][g * _HG:(g + 1) * _HG] for lb in lat], axis=0)
            for t in range(n_expand):
                lhs = jnp.where(own_head, _dot(lg, expand(t)), 0.0).astype(_BF16)
                ctx = ctx + _dot(lhs, head_group(uv0, j * _LANES + t * per_tile, per_tile, g))
                if t % 8 == 7:
                    stream.advance()
        ctx_v[:, g * _HG:(g + 1) * _HG, :] = ctx.reshape(B, _HG, D)

    def project(base):
        tiles = []
        for j in range(hidden_dim // _LANES):
            tiles.append(_dot(xn_lo, column_tile(base, hidden_dim, 0, M, j)))
            if j % 6 == 5:
                stream.advance()
        return tiles

    stream.wait(_WG)
    gate = [jax.nn.silu(v) for v in project(g0)]
    stream.wait(_WU)
    hidden = [(a * v).astype(_BF16) for a, v in zip(gate, project(u0))]
    stream.wait(_WD)
    y = jnp.zeros(x.shape, _F32)
    for j, hj in enumerate(hidden):
        y = y + _dot_nt(hj, column_tile(d0, hidden_dim, 0, M, j))
        if j % 3 == 2:
            stream.advance()
    mixed = jax.nn.silu(xn + (xn * 0.0 + y * route))

    def ctx_rows(h):
        return _pad_rows(ctx_v[:, h, :]).astype(_BF16)

    def per_head(pages):
        for start, size in pages:
            while size:
                h, m_slab = divmod(start, head_slabs)
                n = min(size, head_slabs - m_slab)
                yield h, m_slab * _SLAB, start, n
                start, size = start + n, size - n

    def place(v, m0):
        pads = [jnp.zeros((v.shape[0], w), v.dtype) for w in (m0, M - m0 - v.shape[1])]
        return jnp.concatenate([a for a in (pads[0], v, pads[1]) if a.shape[1]], axis=1)

    lane_tiles = [(m0, min(_LANES, M - m0)) for m0 in range(0, M, _LANES)]
    s = {tile: jnp.zeros((x.shape[0], tile[1]), _F32) for tile in lane_tiles}
    shifted = {}
    for g, pages in enumerate(wo_groups, _WO):
        work = list(per_head(pages))
        lhs = {h: ctx_rows(h) for h in sorted({h for h, _, _, _ in work})}
        stream.wait(g)
        for (m0, _), v in shifted.items():
            wide = place(v, m0)
            s = {(a, w): acc + wide[:, a:a + w] for (a, w), acc in s.items()}
        shifted = {}
        for h, m0, start, n in work:
            tile = (m0, n * _SLAB)
            into = s if tile in s else shifted
            part = _dot_nt(lhs[h], flat(o0 + start, n))
            into[tile] = into[tile] + part if tile in into else part
    assert not shifted

    out = x + jnp.concatenate([s[tile] for tile in lane_tiles], axis=1) * mixed
    out_v[...] = out.astype(out_v.dtype)[:B]
    out_cp = pltpu.make_async_copy(out_v, out_hbm, small_sems.at[0])
    out_cp.start()
    out_cp.wait()


def _slabs(w):
    r, c = w.shape
    w = w.reshape(r // _TILE_ROWS, _TILE_ROWS, c // _LANES, _LANES)
    return w.transpose(0, 2, 1, 3).reshape(-1, _SLAB, _LANES)


@jax.jit
def pallas_recurrent_scan__compressed_kv_cla__moe_arch_mod__decode_kernel(
    A_x: jax.Array,
    A_c_kv: jax.Array,
    A_w_q: jax.Array,
    A_w_uk: jax.Array,
    A_w_uv: jax.Array,
    A_w_o: jax.Array,
    B_x: jax.Array,
    B_w_r: jax.Array,
    B_w_gate: jax.Array,
    B_w_up: jax.Array,
    B_w_down: jax.Array,
):
    del B_x
    B, Sq, M = A_x.shape
    _, Sk, Dc = A_c_kv.shape
    _, H, D = A_w_q.shape
    assert Sq == 1 and H == _SLAB and D == _LANES

    x = A_x.reshape(B, M)
    streamed = [
        A_w_q,
        A_w_uk,
        _slabs(A_c_kv.reshape(B * Sk, Dc)),
        A_w_uv,
        _slabs(B_w_gate),
        _slabs(B_w_up),
        _slabs(B_w_down.T),
        jnp.transpose(A_w_o, (0, 2, 1)).reshape(-1, _SLAB, _LANES),
    ]
    n_slabs = sum(w.shape[0] for w in streamed) + (_HG * _LANES + M * B * _HG * _HG // D) // _SLAB

    def kernel(*refs):
        _kernel(*refs, heads=H, keys=Sk, hidden_dim=B_w_gate.shape[1])

    hbm = pl.BlockSpec(memory_space=pltpu.HBM)
    out = pl.pallas_call(
        kernel,
        out_shape=jax.ShapeDtypeStruct((B, M), A_x.dtype),
        in_specs=[hbm] * (2 + len(streamed)),
        out_specs=hbm,
        scratch_shapes=[
            pltpu.VMEM((n_slabs, _SLAB, _LANES), _BF16),
            pltpu.VMEM(x.shape, x.dtype),
            pltpu.VMEM(B_w_r.shape, B_w_r.dtype),
            pltpu.VMEM(x.shape, x.dtype),
            pltpu.VMEM((B, H, D), _F32),
            pltpu.SemaphoreType.DMA((len(streamed) + len(_WO_GROUPS),)),
            pltpu.SemaphoreType.DMA((2,)),
        ],
        compiler_params=pltpu.CompilerParams(
            vmem_limit_bytes=96 * 1024 * 1024, disable_semaphore_checks=True
        ),
    )(x, B_w_r, *streamed)
    return out.reshape(B, Sq, M)
```

```python
import jax
import jax.numpy as jnp
from jax import lax
import jax.experimental.pallas as pl
import jax.experimental.pallas.tpu as pltpu

_F32 = jnp.float32
_BF16 = jnp.bfloat16
_LANES = 128
_TILE_ROWS = 8
_SLAB = 32
_HG = 16

_WQ, _WUK, _CKV, _WUV, _WG, _WU, _WD, _WO = range(8)

_PAGE = 4
_PAGE_START = 2
_SPACING = (16, 16, 32, 16, 16, 16, 16, 16)
_WO_GROUPS = (36, 12, 8, 4, 4, 4)
_LOW_PER_HIGH = 3
_LEAD = 26
_LOW_AT_END = 20
_STEP = 5
_QUEUE = 82


def _dot(a, b):
    return jnp.dot(a, b, preferred_element_type=_F32)


def _dot_nt(a, b):
    return lax.dot_general(a, b, (((1,), (1,)), ((), ())), preferred_element_type=_F32)


def _iota(shape, axis):
    return lax.broadcasted_iota(jnp.int32, shape, axis)


def _pad_rows(v):
    return jnp.concatenate([v, jnp.zeros((8 - v.shape[0], v.shape[1]), v.dtype)], axis=0)


def _pages(n_slabs, spacing):
    whole = list(range(_PAGE_START, n_slabs - _PAGE + 1, _PAGE))
    ragged = [(whole[-1] + _PAGE, n_slabs), (0, _PAGE_START)]
    return [(a, b - a) for a, b in ragged if b > a] + [
        (start, _PAGE) for i in range(spacing) for start in whole[i::spacing]
    ]


class _Stream:
    def __init__(self, order, groups, buf, sems):
        self.order, self.groups, self.buf, self.sems = order, groups, buf, sems
        is_high = [
            i % (_LOW_PER_HIGH + 1) == 0 and i < len(order) - _LOW_AT_END
            for i in range(len(order))
        ]
        high = [c + (0,) for c, h in zip(order, is_high) if h]
        low = [c + (1,) for c, h in zip(order, is_high) if not h]
        self.todo, low = low[:_LEAD], low[_LEAD:]
        for i, c in enumerate(high):
            self.todo += [c] + low[i * _LOW_PER_HIGH:(i + 1) * _LOW_PER_HIGH]
        self.todo += low[len(high) * _LOW_PER_HIGH:]
        self.ready = {}
        for i, (g, _, _, priority) in enumerate(self.todo):
            self.ready[g] = max(self.ready.get(g, 0), i + (_QUEUE if priority else 8))
        self.done = 0

    def _copy(self, g, start, size):
        src, base = self.groups[g]
        return pltpu.make_async_copy(
            src.at[pl.ds(start, size)], self.buf.at[pl.ds(base + start, size)], self.sems.at[g]
        )

    def advance(self, count=None):
        count = _STEP if count is None else count
        for *copy, priority in self.todo[self.done:self.done + count]:
            self._copy(*copy).start(priority=priority)
        self.done = min(self.done + count, len(self.todo))

    def wait(self, g):
        self.advance(max(self.ready[g] - self.done, 0))
        src, base = self.groups[g]
        copies = [c for c in self.order if c[0] == g]
        if sum(size for _, _, size in copies) == src.shape[0]:
            filled = self.buf.at[pl.ds(base, src.shape[0])]
            pltpu.make_async_copy(filled, filled, self.sems.at[g]).wait()
        else:
            for copy in copies:
                self._copy(*copy).wait()


def _kernel(
    x_hbm, wr_hbm, wq_hbm, wuk_hbm, ckv_hbm, wuv_hbm, wg_hbm, wu_hbm, wd_hbm, wo_hbm,
    out_hbm,
    buf, x_v, wr_v, out_v, ctx_v, sems, small_sems,
    *, heads, keys, hidden_dim,
):
    B, M = x_v.shape
    D = _LANES
    Dc = wuk_hbm.shape[0]
    n_groups = heads // _HG
    rows = B * _HG
    per_tile = _LANES // _HG
    n_expand = _LANES // per_tile

    sources = [wq_hbm, wuk_hbm, ckv_hbm, wuv_hbm, wg_hbm, wu_hbm, wd_hbm, wo_hbm]
    bases = [0]
    for src in sources:
        bases.append(bases[-1] + src.shape[0])
    q0, uk0, kv0, uv0, g0, u0, d0, o0, expand0 = bases
    lhs0 = expand0 + n_expand * _LANES // _SLAB

    groups = list(zip(sources, bases))
    order = [(g, *page) for g in range(_WO) for page in _pages(sources[g].shape[0], _SPACING[g])]
    head_slabs = M // _SLAB
    wo_pages = _pages(wo_hbm.shape[0], _SPACING[_WO])
    last = [
        (start, size) for start, size in wo_pages
        if size == _PAGE and start % head_slabs % _PAGE == 0
        and start % head_slabs + size <= head_slabs
    ][-_LOW_AT_END:]
    wo_pages = [page for page in wo_pages if page not in last] + last
    cuts = [len(wo_pages) - sum(_WO_GROUPS[i:]) for i in range(len(_WO_GROUPS) + 1)]
    wo_groups = [wo_pages[a:b] for a, b in zip([0] + cuts[:-1], cuts)]
    groups += [groups[_WO]] * len(_WO_GROUPS)
    order += [(g, *page) for g, pages in enumerate(wo_groups, _WO) for page in pages]
    stream = _Stream(order, groups, buf, sems)

    def flat(start, n):
        return buf[start:start + n].reshape(n * _SLAB, _LANES)

    def head_group(base, row0, n, g):
        return buf[base + row0:base + row0 + n, g * _HG:(g + 1) * _HG, :].reshape(n * _HG, D)

    per_slab = _SLAB // _TILE_ROWS

    def cache_tile(k0, n, j):
        first = kv0 + k0 // _TILE_ROWS
        tile = slice(j * _TILE_ROWS, (j + 1) * _TILE_ROWS)
        return buf[first:first + n // _TILE_ROWS, tile, :].reshape(n, _LANES)

    def column_tiles(base):
        per_band = hidden_dim // _LANES // per_slab
        for c in range(per_band):
            slabs = [buf[base + i * per_band + c] for i in range(M // _TILE_ROWS)]
            for r in range(0, _SLAB, _TILE_ROWS):
                yield jnp.concatenate([slab[r:r + _TILE_ROWS] for slab in slabs], axis=0)

    def expand(t):
        return flat(expand0 + t * _LANES // _SLAB, _LANES // _SLAB)

    x_cp = pltpu.make_async_copy(x_hbm, x_v, small_sems.at[0])
    wr_cp = pltpu.make_async_copy(wr_hbm, wr_v, small_sems.at[1])
    stream.advance(_LEAD // 2)
    x_cp.start()
    wr_cp.start()
    stream.advance(_QUEUE)

    square = (_LANES, _LANES)
    for t in range(n_expand):
        e = _iota(square, 1) // _HG + t * per_tile == _iota(square, 0)
        first = expand0 + t * _LANES // _SLAB
        buf[first:first + _LANES // _SLAB] = e.astype(_BF16).reshape(-1, _SLAB, _LANES)
        if t % 4 == 3:
            stream.advance()
    own_head = _iota((rows, _LANES), 1) % _HG == _iota((rows, _LANES), 0) % _HG

    x_cp.wait()
    wr_cp.wait()
    x = _pad_rows(x_v[...].astype(_F32))
    xc = x - jnp.mean(x, axis=-1, keepdims=True)
    xn_lo = (xc / jnp.sqrt(jnp.mean(xc * xc, axis=-1, keepdims=True) + 1e-5)).astype(_BF16)
    xn = xn_lo.astype(_F32)
    wr = wr_v[...].astype(_F32).reshape(1, M)
    route = jax.nn.sigmoid(jnp.sum(xn * wr, axis=-1, keepdims=True))

    lhs_slabs = rows // _SLAB
    for t in range(M // per_tile):
        m0 = t // n_expand * _LANES
        n = min(_LANES, M - m0)
        rep = _dot(xn_lo[:, m0:m0 + n], expand(t % n_expand)[:n])
        rep = jnp.concatenate(
            [jnp.broadcast_to(rep[b:b + 1], (_HG, _LANES)) for b in range(B)], axis=0
        )
        first = lhs0 + t * lhs_slabs
        buf[first:first + lhs_slabs] = (
            jnp.where(own_head, rep, 0.0).astype(_BF16).reshape(lhs_slabs, _SLAB, _LANES)
        )
        if t % 8 == 7:
            stream.advance()
    stream.wait(_WQ)
    q = [jnp.zeros((rows, D), _F32) for _ in range(n_groups)]
    for t in range(M // per_tile):
        lhs = flat(lhs0 + t * lhs_slabs, lhs_slabs)
        for g in range(n_groups):
            q[g] = q[g] + _dot(lhs, head_group(q0, t * per_tile, per_tile, g))
        if t % 6 == 5:
            stream.advance()

    stream.wait(_WUK)
    q_lat = []
    for g in range(n_groups):
        qg = q[g].astype(_BF16)
        tiles = []
        for c0 in range(0, Dc, _LANES):
            acc = jnp.zeros((rows, _LANES), _F32)
            for t in range(n_expand):
                full = _dot_nt(qg, head_group(uk0, c0 + t * per_tile, per_tile, g))
                acc = acc + _dot_nt(jnp.where(own_head, full, 0.0).astype(_BF16), expand(t))
                if t % 8 == 7:
                    stream.advance()
            tiles.append(acc.astype(_BF16))
        q_lat.append(tiles)

    qk_keys, pv_keys = 512, 1024
    lat_tiles = range(Dc // _LANES)

    def scores(b):
        qb = [
            jnp.concatenate([q_lat[g][j][b * _HG:(b + 1) * _HG] for g in range(n_groups)], axis=0)
            for j in lat_tiles
        ]
        chunks = []
        for k0 in range(b * keys, (b + 1) * keys, qk_keys):
            parts = [_dot_nt(qb[j], cache_tile(k0, qk_keys, j)) for j in lat_tiles]
            chunks.append(sum(parts[1:], parts[0]))
            stream.advance()
        return jnp.concatenate(chunks, axis=1) * (D ** -0.5)

    def attend(b, s):
        p = jnp.exp(s - jnp.max(s, axis=-1, keepdims=True))
        denom = jnp.sum(p, axis=-1, keepdims=True)
        p = p.astype(_BF16)
        acc = [jnp.zeros((heads, _LANES), _F32) for _ in lat_tiles]
        for k0 in range(0, keys, pv_keys):
            acc = [
                a + _dot(p[:, k0:k0 + pv_keys], cache_tile(b * keys + k0, pv_keys, j))
                for j, a in enumerate(acc)
            ]
            stream.advance()
        return [(a / denom).astype(_BF16) for a in acc]

    stream.wait(_CKV)
    lat = []
    s = scores(0)
    for b in range(B):
        ahead = scores(b + 1) if b + 1 < B else None
        lat.append(attend(b, s))
        s = ahead

    stream.wait(_WUV)
    for g in range(n_groups):
        ctx = jnp.zeros((rows, D), _F32)
        for j in range(Dc // _LANES):
            lg = jnp.concatenate([lb[j][g * _HG:(g + 1) * _HG] for lb in lat], axis=0)
            for t in range(n_expand):
                lhs = jnp.where(own_head, _dot(lg, expand(t)), 0.0).astype(_BF16)
                ctx = ctx + _dot(lhs, head_group(uv0, j * _LANES + t * per_tile, per_tile, g))
                if t % 8 == 7:
                    stream.advance()
        ctx_v[:, g * _HG:(g + 1) * _HG, :] = ctx.reshape(B, _HG, D)

    def project(base):
        tiles = []
        for j, w in enumerate(column_tiles(base)):
            tiles.append(_dot(xn_lo, w))
            if j % 6 == 5:
                stream.advance()
        return tiles

    stream.wait(_WG)
    gate = [jax.nn.silu(v) for v in project(g0)]
    stream.wait(_WU)
    hidden = [(a * v).astype(_BF16) for a, v in zip(gate, project(u0))]
    stream.wait(_WD)
    y = jnp.zeros(x.shape, _F32)
    for j, w in enumerate(column_tiles(d0)):
        y = y + _dot_nt(hidden[j], w)
        if j % 3 == 2:
            stream.advance()
    mixed = jax.nn.silu(xn + (xn * 0.0 + y * route))

    def ctx_rows(h):
        return _pad_rows(ctx_v[:, h, :]).astype(_BF16)

    def per_head(pages):
        for start, size in pages:
            while size:
                h, m_slab = divmod(start, head_slabs)
                n = min(size, head_slabs - m_slab)
                yield h, m_slab * _SLAB, start, n
                start, size = start + n, size - n

    def place(v, m0):
        pads = [jnp.zeros((v.shape[0], w), v.dtype) for w in (m0, M - m0 - v.shape[1])]
        return jnp.concatenate([a for a in (pads[0], v, pads[1]) if a.shape[1]], axis=1)

    lane_tiles = [(m0, min(_LANES, M - m0)) for m0 in range(0, M, _LANES)]
    s = {tile: jnp.zeros((x.shape[0], tile[1]), _F32) for tile in lane_tiles}
    shifted = {}
    for g, pages in enumerate(wo_groups, _WO):
        work = list(per_head(pages))
        lhs = {h: ctx_rows(h) for h in sorted({h for h, _, _, _ in work})}
        stream.wait(g)
        for (m0, _), v in shifted.items():
            wide = place(v, m0)
            s = {(a, w): acc + wide[:, a:a + w] for (a, w), acc in s.items()}
        shifted = {}
        for h, m0, start, n in work:
            tile = (m0, n * _SLAB)
            into = s if tile in s else shifted
            part = _dot_nt(lhs[h], flat(o0 + start, n))
            into[tile] = into[tile] + part if tile in into else part
    assert not shifted

    out = x + jnp.concatenate([s[tile] for tile in lane_tiles], axis=1) * mixed
    out_v[...] = out.astype(out_v.dtype)[:B]
    out_cp = pltpu.make_async_copy(out_v, out_hbm, small_sems.at[0])
    out_cp.start()
    out_cp.wait()


def _slabs(w):
    r, c = w.shape
    w = w.reshape(r // _TILE_ROWS, _TILE_ROWS, c // _LANES, _LANES)
    return w.transpose(0, 2, 1, 3).reshape(-1, _SLAB, _LANES)


@jax.jit
def pallas_recurrent_scan__compressed_kv_cla__moe_arch_mod__decode_kernel(
    A_x: jax.Array,
    A_c_kv: jax.Array,
    A_w_q: jax.Array,
    A_w_uk: jax.Array,
    A_w_uv: jax.Array,
    A_w_o: jax.Array,
    B_x: jax.Array,
    B_w_r: jax.Array,
    B_w_gate: jax.Array,
    B_w_up: jax.Array,
    B_w_down: jax.Array,
):
    del B_x
    B, Sq, M = A_x.shape
    _, Sk, Dc = A_c_kv.shape
    _, H, D = A_w_q.shape
    assert Sq == 1 and H == _SLAB and D == _LANES

    x = A_x.reshape(B, M)
    streamed = [
        A_w_q,
        A_w_uk,
        _slabs(A_c_kv.reshape(B * Sk, Dc)),
        A_w_uv,
        _slabs(B_w_gate),
        _slabs(B_w_up),
        _slabs(B_w_down.T),
        jnp.transpose(A_w_o, (0, 2, 1)).reshape(-1, _SLAB, _LANES),
    ]
    n_slabs = sum(w.shape[0] for w in streamed) + (_HG * _LANES + M * B * _HG * _HG // D) // _SLAB

    def kernel(*refs):
        _kernel(*refs, heads=H, keys=Sk, hidden_dim=B_w_gate.shape[1])

    hbm = pl.BlockSpec(memory_space=pltpu.HBM)
    out = pl.pallas_call(
        kernel,
        out_shape=jax.ShapeDtypeStruct((B, M), A_x.dtype),
        in_specs=[hbm] * (2 + len(streamed)),
        out_specs=hbm,
        scratch_shapes=[
            pltpu.VMEM((n_slabs, _SLAB, _LANES), _BF16),
            pltpu.VMEM(x.shape, x.dtype),
            pltpu.VMEM(B_w_r.shape, B_w_r.dtype),
            pltpu.VMEM(x.shape, x.dtype),
            pltpu.VMEM((B, H, D), _F32),
            pltpu.SemaphoreType.DMA((len(streamed) + len(_WO_GROUPS),)),
            pltpu.SemaphoreType.DMA((2,)),
        ],
        compiler_params=pltpu.CompilerParams(
            vmem_limit_bytes=96 * 1024 * 1024, disable_semaphore_checks=True
        ),
    )(x, B_w_r, *streamed)
    return out.reshape(B, Sq, M)
```
